```python
import jax
import jax.numpy as jnp

def _softmax(x, axis=-1):
    return jax.nn.softmax(x, axis=axis)
def _gelu(x):
    return jax.nn.gelu(x, approximate=True)
def _silu(x):
    return jax.nn.silu(x)
def _sigmoid(x):
    return jax.nn.sigmoid(x)
def _layernorm(x, axis=-1, eps=1e-5):
    m = jnp.mean(x, axis=axis, keepdims=True)
    v = jnp.var(x, axis=axis, keepdims=True)
    return (x - m) / jnp.sqrt(v + eps)
def _scatter_add(tgt, idx, src, axis=0):
    return tgt.at[idx].add(src)
def _segment_sum(src, seg, n):
    return jax.ops.segment_sum(src, seg, n)
class _Rng:
    def __init__(self, key):
        self._k = key
    def _next(self):
        self._k, sub = jax.random.split(self._k)
        return sub
    def normal(self, shape):
        return jax.random.normal(self._next(), shape, dtype=jnp.bfloat16)
    def randint(self, lo, hi, shape):
        return jax.random.randint(self._next(), shape, lo, hi, dtype=jnp.int32)
    def uniform(self, shape, lo=0.0, hi=1.0):
        return jax.random.uniform(self._next(), shape, jnp.bfloat16, lo, hi)
    def permutation(self, n):
        return jax.random.permutation(self._next(), n)


kernel_name = 'concat_heads__compressed_kv_cla__mha_block_cached__decode'

def setup_inputs():
    _rng = _Rng(jax.random.key(int.from_bytes(__import__("os").urandom(4), "little")))
    _w = (lambda a: (lambda t: t.astype(jnp.bfloat16) if jnp.issubdtype(t.dtype, jnp.floating) else t)(jnp.asarray(a)))
    def _A_setup():
        B, H, Sq, Sk, D, M = 4, 32, 1, 4096, 128, 512
        Dc = 4 * D
        return {
            "x": _w((lambda *s: _rng.normal(s) * 0.05)(B, Sq, M)),
            "c_kv": _w((lambda *s: _rng.normal(s) * 0.05)(B, Sk, Dc)),
            "w_q": _w((lambda *s: _rng.normal(s) * 0.05)(M, H, D) * (M ** -0.5)),
            "w_uk": _w((lambda *s: _rng.normal(s) * 0.05)(Dc, H, D) * (Dc ** -0.5)),
            "w_uv": _w((lambda *s: _rng.normal(s) * 0.05)(Dc, H, D) * (Dc ** -0.5)),
            "w_o": _w((lambda *s: _rng.normal(s) * 0.05)(H, D, M) * ((H * D) ** -0.5)),
        }
    _A_in = _A_setup()

    def _B_setup():
        B, Sq, D = 4, 1, 512
        H, Sk, Dh = 32, 4096, 128
        return {
            "x": _w((lambda *s: _rng.normal(s) * 0.05)(B, Sq, D)),
            "k_cache": _w((lambda *s: _rng.normal(s) * 0.05)(B, H, Sk, Dh)),
            "v_cache": _w((lambda *s: _rng.normal(s) * 0.05)(B, H, Sk, Dh)),
            "wq": _w((lambda *s: _rng.normal(s) * 0.05)(D, H * Dh) * (D ** -0.5)),
            "wo": _w((lambda *s: _rng.normal(s) * 0.05)(H * Dh, D) * ((H * Dh) ** -0.5)),
        }
    _B_in = _B_setup()

    return {
        "A_x": _A_in["x"],
        "A_c_kv": _A_in["c_kv"],
        "A_w_q": _A_in["w_q"],
        "A_w_uk": _A_in["w_uk"],
        "A_w_uv": _A_in["w_uv"],
        "A_w_o": _A_in["w_o"],
        "B_x": _B_in["x"],
        "B_k_cache": _B_in["k_cache"],
        "B_v_cache": _B_in["v_cache"],
        "B_wq": _B_in["wq"],
        "B_wo": _B_in["wo"],
    }

def reference(A_x, A_c_kv, A_w_q, A_w_uk, A_w_uv, A_w_o, B_x, B_k_cache, B_v_cache, B_wq, B_wo):
    def _A_ref(x, c_kv, w_q, w_uk, w_uv, w_o):
        B, Sq, M = x.shape[0], x.shape[1], x.shape[2]
        Sk = c_kv.shape[1]
        H, D = w_q.shape[1], w_q.shape[2]
        q = jnp.einsum("bqm,mhd->bhqd", x, w_q)
        k = jnp.einsum("bkc,chd->bhkd", c_kv, w_uk)
        v = jnp.einsum("bkc,chd->bhkd", c_kv, w_uv)
        scores = jnp.einsum("bhqd,bhkd->bhqk", q, k) * (D ** -0.5)
        off = Sk - Sq
        qi = jnp.arange(Sq)[:, None]
        kj = jnp.arange(Sk)[None, :]
        cmask = kj <= (qi + off)
        scores = jnp.where(cmask[None, None], scores, -1e9)
        p = _softmax(scores, axis=-1)
        ctx = jnp.einsum("bhqk,bhkd->bhqd", p, v)
        return jnp.einsum("bhqd,hdm->bqm", ctx, w_o)

    def _B_ref(x, k_cache, v_cache, wq, wo):
        B, Sq, D = x.shape
        H, Dh = 32, 128
        q = (lambda x, *d: x.transpose(*d))((x @ wq).reshape(B, Sq, H, Dh), 0, 2, 1, 3)
        scores = jnp.einsum("bhqd,bhkd->bhqk", q, k_cache) * (Dh ** -0.5)
        p = _softmax(scores, axis=-1)
        o = jnp.einsum("bhqk,bhkd->bhqd", p, v_cache)
        return (lambda x, *d: x.transpose(*d))(o, 0, 2, 1, 3).reshape(B, Sq, H * Dh) @ wo

    a = _A_ref(A_x, A_c_kv, A_w_q, A_w_uk, A_w_uv, A_w_o)
    b = _B_ref(B_x, B_k_cache, B_v_cache, B_wq, B_wo)
    return jnp.concatenate([a, b], axis=-1)
```

```python
import math

import jax
import jax.numpy as jnp
from jax import lax
import jax.experimental.pallas as pl
import jax.experimental.pallas.tpu as pltpu

F32 = jnp.float32
BF16 = jnp.bfloat16
NT = (((1,), (1,)), ((), ()))

NB, NH, SK, HD, DM = 4, 32, 4096, 128, 512
BLOCK = 64 * 1024
NS = 8
NR = 8
LAG = 3
A_HEAD = 32 * 1024
B_HEAD = 48 * 1024
HG = 8


def _aligned(x, m):
    return x if isinstance(x, int) else pl.multiple_of(x, m)


def _loop(n, body, init=None, lo=0):
    return lax.fori_loop(lo, n, body, init)


def _when(cond, fn):
    if cond is True:
        fn()
    elif cond is not False:
        pl.when(cond)(fn)


def _kernel(ax_hbm, ckv_hbm, wq_hbm, wuk_hbm, wuv_hbm, wo_hbm, bx_hbm, k_hbm, v_hbm, bwq_hbm, bwo_hbm,
            out_ref,
            ax_v, bx_v, ckv_v, wq_v, wuk_v, wuv_v, wo_v, bwq_v, bwo_v, k_v, v_v,
            e_v, lat_v, head_v, sa_v, qb_v, sb_v, cb_v,
            x_sem, w_sem, ckv_sem, k_sem, v_sem, bwo_sem):
    scale = HD ** -0.5
    bwq_sem, wq_sem, wuk_sem, wuv_sem, wo_sem = (w_sem.at[i] for i in range(5))

    def wait_all(dst, sem):
        pltpu.make_async_copy(dst, dst, sem).wait()

    def piece(rows, tail, split=B_HEAD):
        head = rows * split // BLOCK
        return (head, rows - head) if tail else (0, head)

    def block(first, s, r, tail):
        if not tail:
            return first(s) + r
        jump = first((s - 1) % NS) + NR - first(s)
        return first(s) + r - 1 + (jnp.where(r == 0, jump, 0) if jump else 0)

    def matrix(src, dst, sem, base=0):
        def copy(s, r, tail):
            rows = BLOCK // (2 * math.prod(src.shape[1:]))
            off, size = piece(rows, tail, A_HEAD)
            at = pl.ds(_aligned(base + block(lambda i: i * NR, s, r, tail) * rows + off, rows // 4), size)
            return pltpu.make_async_copy(src.at[at], dst.at[at], sem)
        return copy

    def cache(src, dst, sem, h):
        def copy(s, r, tail):
            rows = BLOCK // (2 * HD)
            off, size = piece(rows, tail)
            n = block(lambda i: i // 2 * NH * 2 * NR + i % 2 * NR, s, r, tail)
            m = block(lambda i: i * NR, s, r, tail)
            return pltpu.make_async_copy(src.at[pl.ds(_aligned(h * SK + n * rows + off, 16), size)],
                                         dst.at[h & 1, pl.ds(_aligned(m * rows + off, 16), size)], sem.at[h & 1])
        return copy

    def bwq(s, r, tail):
        n = block(lambda i: i * NR, s, r, tail)
        cols = pl.ds(*piece(NH * HD, tail))
        return pltpu.make_async_copy(bwq_hbm.at[pl.ds(_aligned(n * 8, 8), 8), cols], bwq_v.at[n, :, cols], bwq_sem)

    def bwo(s, r, tail):
        n = block(lambda i: i * NR, s, r, tail)
        rows = BLOCK // (2 * DM)
        off, size = piece(rows, tail)
        s, i = n >> 3, (n >> 1) & 3
        return pltpu.make_async_copy(bwo_hbm.at[pl.ds(_aligned(n * rows + off, 16), size)],
                                     bwo_v.at[i, s, pl.ds(_aligned((n & 1) * rows + off, 16), size)],
                                     bwo_sem.at[jnp.where(i < 3, i, 3 + s)])

    def ckv(b):
        return matrix(ckv_hbm, ckv_v, ckv_sem.at[b], b * SK)

    def k_cache(h):
        return cache(k_hbm, k_v, k_sem, h)

    def v_cache(h):
        return cache(v_hbm, v_v, v_sem, h)

    wq, wuk = matrix(wq_hbm, wq_v, wq_sem), matrix(wuk_hbm, wuk_v, wuk_sem)
    wuv, wo = matrix(wuv_hbm, wuv_v, wuv_sem), matrix(wo_hbm, wo_v, wo_sem)

    def start_round(r, unit, previous):
        def start(tails, round_):
            for s in range(NS):
                if tails is not None:
                    tails(s, round_, True).start(priority=0)
                unit(s, r, False).start(priority=1)

        pl.when(r < LAG)(lambda: start(previous, r + NR - LAG))
        pl.when(r >= LAG)(lambda: start(unit, r - LAG))

    row8 = lax.broadcasted_iota(jnp.int32, (8, HD), 0) & (NB - 1)
    group = NB * HG

    def same_head(rows):
        r = lax.broadcasted_iota(jnp.int32, (rows, HD * HG), 0)
        l = lax.broadcasted_iota(jnp.int32, (rows, HD * HG), 1)
        return (r & (HG - 1)) == (l & (HG - 1))

    def weights(w_ref, r, i):
        c = pl.ds(_aligned((r & 3) * HD, HD), HD)
        h = pl.ds(_aligned(((r >> 2) * 2 + i) * HG, HG), HG)
        return w_ref[c, h, :].reshape(HD * HG, HD)

    def two_groups(r):
        return pl.ds(_aligned((r >> 2) * 2 * group, 2 * group), 2 * group)

    def up_project(w_ref, r, acc):
        wide = jnp.dot(lat_v[r & 3, two_groups(r), :].astype(BF16), e_v[...], preferred_element_type=F32)
        wide = jnp.where(same_head(2 * group), wide, 0.0).astype(BF16)
        acc = acc + jnp.concatenate([jnp.dot(wide[i * group:(i + 1) * group], weights(w_ref, r, i),
                                             preferred_element_type=F32) for i in range(2)], axis=0)
        head_v[two_groups(r), :] = acc
        return jnp.where((r & 3) == 3, 0.0, acc)

    x_copies = [pltpu.make_async_copy(ax_hbm, ax_v, x_sem.at[0]), pltpu.make_async_copy(bx_hbm, bx_v, x_sem.at[1])]

    def setup(r, _):
        start_round(r, bwq, None)
        c = lax.broadcasted_iota(jnp.int32, (HD // NR, HD * HG), 0) + r * (HD // NR)
        l = lax.broadcasted_iota(jnp.int32, (HD // NR, HD * HG), 1) >> 3
        e_v[pl.ds(_aligned(r * (HD // NR), HD // NR), HD // NR), :] = jnp.where(c == l, 1.0, 0.0).astype(BF16)

    _loop(NR, setup)
    for copy in x_copies:
        copy.start()
    _loop(NR, lambda r, _: start_round(r, wq, bwq))
    for copy in x_copies:
        copy.wait()
    xa = ax_v[...].astype(F32)
    for b in range(NB):
        for j in range(DM // HD):
            for g in range(NH // HG):
                lat_v[j, pl.ds(g * group + b * HG, HG), :] = jnp.broadcast_to(xa[b:b + 1, j * HD:(j + 1) * HD], (HG, HD))
    xb = bx_v[...].astype(F32)
    xb = jnp.concatenate([xb, xb], axis=0).astype(BF16)

    def b_queries(r, _):
        start_round(r, wuk, wq)
        cols = NH * HD // NR
        w = bwq_v[:, :, pl.ds(_aligned(r * cols, cols), cols)].reshape(DM, cols)
        q = jnp.dot(xb, w, preferred_element_type=F32)
        for k in range(NH // NR):
            qb_v[r * (NH // NR) + k] = q[:, k * HD:(k + 1) * HD]

    wait_all(bwq_v, bwq_sem)
    _loop(NR, b_queries)

    def a_queries(r, acc):
        start_round(r, ckv(0), wuk)
        return up_project(wq_v, r, acc)

    wait_all(wq_v, wq_sem)
    _loop(NR, a_queries, jnp.zeros((2 * group, HD), F32))

    def a_absorb(r, _):
        start_round(r, ckv(1), ckv(0))
        q = head_v[two_groups(r), :].astype(BF16)
        wide = jnp.concatenate([lax.dot_general(q[i * group:(i + 1) * group], weights(wuk_v, r, i), NT,
                                                preferred_element_type=F32) for i in range(2)], axis=0)
        wide = jnp.where(same_head(2 * group), wide, 0.0).astype(BF16)
        lat_v[r & 3, two_groups(r), :] = lax.dot_general(wide, e_v[...], NT, preferred_element_type=F32)

    wait_all(wuk_v, wuk_sem)
    _loop(NR, a_absorb)

    def a_attention(b, _):
        half = NR // 2
        keys = SK // half

        def start(r):
            pl.when(b < 2)(lambda: start_round(r, ckv(b + 2), ckv(b + 1)))
            pl.when(b == 2)(lambda: start_round(r, wuv, ckv(3)))
            pl.when(b == 3)(lambda: start_round(r, k_cache(0), wuv))

        def latents(i):
            return ckv_v[pl.ds(_aligned(b * SK + i * keys, keys), keys), :]

        heads = [pl.ds(_aligned(g * group + b * HG, HG), HG) for g in range(NH // HG)]
        q = jnp.concatenate([jnp.concatenate([lat_v[j, g, :] for g in heads], axis=0)
                             for j in range(DM // HD)], axis=1).astype(BF16)

        def scores(i, m):
            start(i)
            s = lax.dot_general(q, latents(i), NT, preferred_element_type=F32) * scale
            sa_v[i] = s
            return jnp.maximum(m, jnp.max(s, axis=-1, keepdims=True))

        def context(i, carry):
            start(half + i)
            p = jnp.exp(sa_v[i] - m)
            c = jnp.dot(p.astype(BF16), latents(i), preferred_element_type=F32)
            return carry[0] + c, carry[1] + jnp.sum(p, axis=-1, keepdims=True)

        wait_all(ckv_v.at[pl.ds(_aligned(b * SK, SK), SK)], ckv_sem.at[b])
        m = _loop(half, scores, jnp.full((NH, 1), -jnp.inf, F32))
        c, l = _loop(half, context, (jnp.zeros((NH, DM), F32), jnp.zeros((NH, 1), F32)))
        c = c / l
        for j in range(DM // HD):
            for g in range(NH // HG):
                lat_v[j, heads[g], :] = c[g * HG:(g + 1) * HG, j * HD:(j + 1) * HD]

    _loop(NB, a_attention)

    def a_values(r, acc):
        start_round(r, v_cache(0), k_cache(0))
        return up_project(wuv_v, r, acc)

    wait_all(wuv_v, wuv_sem)
    _loop(NR, a_values, jnp.zeros((2 * group, HD), F32))

    keys = SK // NR

    def b_head(h, _):
        q = qb_v[h].astype(BF16)

        def tile(ref, r, b):
            return ref[h & 1, pl.ds(_aligned(b * SK + r * keys, keys), keys), :]

        def scores(r, m):
            pl.when(h + 1 < NH)(lambda: start_round(r, k_cache(h + 1), v_cache(h)))
            pl.when(h + 1 == NH)(lambda: start_round(r, wo, v_cache(NH - 1)))
            row = lax.broadcasted_iota(jnp.int32, (8, keys), 0) % NB
            s = None
            for b in range(NB):
                d = lax.dot_general(q, tile(k_v, r, b), NT, preferred_element_type=F32)
                s = d if s is None else jnp.where(row == b, d, s)
            s = s * scale
            sb_v[r] = s
            return jnp.maximum(m, s)

        def context(r, carry):
            pl.when(h + 1 < NH)(lambda: start_round(r, v_cache(h + 1), k_cache(h + 1)))
            pl.when(h + 1 == NH)(lambda: start_round(r, bwo, wo))
            ctx, l = carry
            p = jnp.exp(sb_v[r] - m)
            for b in range(NB):
                d = jnp.dot(p.astype(BF16), tile(v_v, r, b), preferred_element_type=F32)
                ctx = ctx + jnp.where(row8 == b, d, 0.0)
            return ctx, l + p

        wait_all(k_v.at[h & 1], k_sem.at[h & 1])
        m = jnp.max(_loop(NR, scores, jnp.full((8, keys), -jnp.inf, F32)), axis=-1, keepdims=True)
        wait_all(v_v.at[h & 1], v_sem.at[h & 1])
        ctx, l = _loop(NR, context, (jnp.zeros((8, HD), F32), jnp.zeros((8, keys), F32)))
        cb_v[h] = ctx / jnp.sum(l, axis=-1, keepdims=True)

    _loop(NH, b_head)

    def b_output(i, s):
        return jnp.dot(cb_v[s * (NH // NS) + i].astype(BF16), bwo_v[i, s], preferred_element_type=F32)

    def outputs(k, carry):
        for i in range(LAG):
            n = k * LAG + i
            bwo(0, (n & 7) * NR + NR - LAG + (n >> 3), True).start(priority=0)

        @pl.when((k & 3) == 0)
        def _():
            wait_all(bwo_v.at[k >> 2], bwo_sem.at[k >> 2])

        ctx = head_v[pl.ds(_aligned((k >> 1) * group, group), group), :]
        head = lax.broadcasted_iota(jnp.int32, (group, HD), 0) & (HG - 1)
        lhs = jnp.concatenate([jnp.where(head == (k & 1) * 4 + i, ctx, 0.0) for i in range(4)], axis=1)
        w = wo_v[pl.ds(_aligned(k * DM, DM), DM), :]
        return (carry[0] + jnp.dot(lhs.astype(BF16), w, preferred_element_type=F32),
                carry[1] + b_output(k >> 2, (k & 3) * 2) + b_output(k >> 2, (k & 3) * 2 + 1))

    wait_all(wo_v, wo_sem)
    out_a, out_b = _loop(NR, outputs, (jnp.zeros((group, DM), F32), jnp.zeros((8, DM), F32)))
    out_ref[:, pl.ds(0, DM)] = jnp.concatenate(
        [jnp.sum(out_a[b * HG:(b + 1) * HG], axis=0, keepdims=True) for b in range(NB)], axis=0).astype(out_ref.dtype)

    wait_all(bwo_v.at[2], bwo_sem.at[2])
    for s in range(NS):
        out_b = out_b + b_output(2, s)
    for s in range(NS):
        wait_all(bwo_v.at[3, s], bwo_sem.at[3 + s])
        out_b = out_b + b_output(3, s)
    out_ref[:, pl.ds(DM, DM)] = out_b[:NB].astype(out_ref.dtype)


@jax.jit
def pallas_concat_heads__compressed_kv_cla__mha_block_cached__decode_kernel(
    A_x: jax.Array,
    A_c_kv: jax.Array,
    A_w_q: jax.Array,
    A_w_uk: jax.Array,
    A_w_uv: jax.Array,
    A_w_o: jax.Array,
    B_x: jax.Array,
    B_k_cache: jax.Array,
    B_v_cache: jax.Array,
    B_wq: jax.Array,
    B_wo: jax.Array,
):
    assert A_x.shape == (NB, 1, DM) and A_c_kv.shape == (NB, SK, DM) and A_w_q.shape == (DM, NH, HD)
    assert B_x.shape == (NB, 1, DM) and B_k_cache.shape == (NB, NH, SK, HD)
    scratch = [
        pltpu.VMEM((NB, DM), BF16),
        pltpu.VMEM((NB, DM), BF16),
        pltpu.VMEM((NB * SK, DM), BF16),
        pltpu.VMEM((DM, NH, HD), BF16),
        pltpu.VMEM((DM, NH, HD), BF16),
        pltpu.VMEM((DM, NH, HD), BF16),
        pltpu.VMEM((NH * HD, DM), BF16),
        pltpu.VMEM((DM // 8, 8, NH * HD), BF16),
        pltpu.VMEM((NH // NS, NS, HD, DM), BF16),
        pltpu.VMEM((2, NB * SK, HD), BF16),
        pltpu.VMEM((2, NB * SK, HD), BF16),
        pltpu.VMEM((HD, HD * HG), BF16),
        pltpu.VMEM((DM // HD, NB * NH, HD), F32),
        pltpu.VMEM((NB * NH, HD), F32),
        pltpu.VMEM((NR // 2, NH, 2 * SK // NR), F32),
        pltpu.VMEM((NH, 8, HD), F32),
        pltpu.VMEM((NR, 8, SK // NR), F32),
        pltpu.VMEM((NH, 8, HD), F32),
        pltpu.SemaphoreType.DMA((2,)),
        pltpu.SemaphoreType.DMA((5,)),
        pltpu.SemaphoreType.DMA((NB,)),
        pltpu.SemaphoreType.DMA((2,)),
        pltpu.SemaphoreType.DMA((2,)),
        pltpu.SemaphoreType.DMA((3 + NS,)),
    ]
    out = pl.pallas_call(
        _kernel,
        out_shape=jax.ShapeDtypeStruct((NB, 2 * DM), A_x.dtype),
        in_specs=[pl.BlockSpec(memory_space=pl.ANY)] * 11,
        out_specs=pl.BlockSpec(memory_space=pltpu.VMEM),
        scratch_shapes=scratch,
        compiler_params=pltpu.CompilerParams(vmem_limit_bytes=100 * 1024 * 1024, disable_bounds_checks=True),
    )(
        A_x.reshape(NB, DM),
        A_c_kv.reshape(NB * SK, DM),
        A_w_q,
        A_w_uk,
        A_w_uv,
        A_w_o.reshape(NH * HD, DM),
        B_x.reshape(NB, DM),
        B_k_cache.reshape(NB * NH * SK, HD),
        B_v_cache.reshape(NB * NH * SK, HD),
        B_wq,
        B_wo,
    )
    return out.reshape(NB, 1, 2 * DM)
```

```python
import math

import jax
import jax.numpy as jnp
from jax import lax
import jax.experimental.pallas as pl
import jax.experimental.pallas.tpu as pltpu

F32 = jnp.float32
BF16 = jnp.bfloat16
NT = (((1,), (1,)), ((), ()))

NB, NH, SK, HD, DM = 4, 32, 4096, 128, 512
BLOCK = 64 * 1024
NS = 8
NR = 8
LAG = 26
A_HEAD = 32 * 1024
B_HEAD = 48 * 1024
LAST = ((0, 1, 2, 3), (4, 5), (6, 7))
NOCHECK = True
HG = 8


def _aligned(x, m):
    return x if isinstance(x, int) else pl.multiple_of(x, m)


def _loop(n, body, init=None, lo=0):
    return lax.fori_loop(lo, n, body, init)


def _when(cond, fn):
    if cond is True:
        fn()
    elif cond is not False:
        pl.when(cond)(fn)


def _kernel(ax_hbm, ckv_hbm, wq_hbm, wuk_hbm, wuv_hbm, wo_hbm, bx_hbm, k_hbm, v_hbm, bwq_hbm, bwo_hbm,
            out_ref,
            ax_v, bx_v, ckv_v, wq_v, wuk_v, wuv_v, wo_v, bwq_v, bwo_v, k_v, v_v,
            e_v, lat_v, head_v, sa_v, qb_v, sb_v, cb_v,
            x_sem, w_sem, ckv_sem, k_sem, v_sem, bwo_sem):
    scale = HD ** -0.5
    bwq_sem, wq_sem, wuk_sem, wuv_sem, wo_sem = (w_sem.at[i] for i in range(5))

    def wait_all(dst, sem):
        pltpu.make_async_copy(dst, dst, sem).wait()

    def piece(rows, tail, split=B_HEAD):
        head = rows * split // BLOCK
        return (head, rows - head) if tail else (0, head)

    def block(first, s, r, tail):
        if not tail:
            return first(s) + r
        jump = first((s - 1) % NS) + NR - first(s)
        return first(s) + r - 1 + (jnp.where(r == 0, jump, 0) if jump else 0)

    def matrix(src, dst, sem, base=0):
        def copy(s, r, tail):
            rows = BLOCK // (2 * math.prod(src.shape[1:]))
            off, size = piece(rows, tail, A_HEAD)
            at = pl.ds(_aligned(base + block(lambda i: i * NR, s, r, tail) * rows + off, rows // 4), size)
            return pltpu.make_async_copy(src.at[at], dst.at[at], sem)
        return copy

    def cache(src, dst, sem, h):
        def copy(s, r, tail):
            rows = BLOCK // (2 * HD)
            off, size = piece(rows, tail)
            n = block(lambda i: i // 2 * NH * 2 * NR + i % 2 * NR, s, r, tail)
            m = block(lambda i: i * NR, s, r, tail)
            return pltpu.make_async_copy(src.at[pl.ds(_aligned(h * SK + n * rows + off, 16), size)],
                                         dst.at[h & 1, pl.ds(_aligned(m * rows + off, 16), size)], sem.at[h & 1])
        return copy

    def bwq(s, r, tail):
        n = block(lambda i: i * NR, s, r, tail)
        cols = pl.ds(*piece(NH * HD, tail))
        return pltpu.make_async_copy(bwq_hbm.at[pl.ds(_aligned(n * 8, 8), 8), cols], bwq_v.at[n, :, cols], bwq_sem)

    def bwo(s, r, tail):
        n = block(lambda i: i * NR, s, r, tail)
        rows = BLOCK // (2 * DM)
        off, size = piece(rows, tail)
        s, i = n >> 3, (n >> 1) & 3
        return pltpu.make_async_copy(bwo_hbm.at[pl.ds(_aligned(n * rows + off, 16), size)],
                                     bwo_v.at[i, s, pl.ds(_aligned((n & 1) * rows + off, 16), size)],
                                     bwo_sem.at[jnp.where(i < 3, i, 3 + s)])

    def ckv(b):
        return matrix(ckv_hbm, ckv_v, ckv_sem.at[b], b * SK)

    def k_cache(h):
        return cache(k_hbm, k_v, k_sem, h)

    def v_cache(h):
        return cache(v_hbm, v_v, v_sem, h)

    wq, wuk = matrix(wq_hbm, wq_v, wq_sem), matrix(wuk_hbm, wuk_v, wuk_sem)
    wuv, wo = matrix(wuv_hbm, wuv_v, wuv_sem), matrix(wo_hbm, wo_v, wo_sem)

    def start_round(r, unit, previous):
        for streams in (range(LAG % NS), range(LAG % NS, NS)):
            if not streams:
                continue
            back = -((streams[0] - LAG) // NS)

            def start(tails, round_):
                for s in streams:
                    if tails is not None:
                        tails((s - LAG) % NS, round_, True).start(priority=0)
                    unit(s, r, False).start(priority=1)

            pl.when(r < back)(lambda: start(previous, r + NR - back))
            pl.when(r >= back)(lambda: start(unit, r - back))

    row8 = lax.broadcasted_iota(jnp.int32, (8, HD), 0) & (NB - 1)
    group = NB * HG

    def same_head(rows):
        r = lax.broadcasted_iota(jnp.int32, (rows, HD * HG), 0)
        l = lax.broadcasted_iota(jnp.int32, (rows, HD * HG), 1)
        return (r & (HG - 1)) == (l & (HG - 1))

    def weights(w_ref, r, i):
        c = pl.ds(_aligned((r & 3) * HD, HD), HD)
        h = pl.ds(_aligned(((r >> 2) * 2 + i) * HG, HG), HG)
        return w_ref[c, h, :].reshape(HD * HG, HD)

    def two_groups(r):
        return pl.ds(_aligned((r >> 2) * 2 * group, 2 * group), 2 * group)

    def up_project(w_ref, r, acc):
        wide = jnp.dot(lat_v[r & 3, two_groups(r), :].astype(BF16), e_v[...], preferred_element_type=F32)
        wide = jnp.where(same_head(2 * group), wide, 0.0).astype(BF16)
        acc = acc + jnp.concatenate([jnp.dot(wide[i * group:(i + 1) * group], weights(w_ref, r, i),
                                             preferred_element_type=F32) for i in range(2)], axis=0)
        head_v[two_groups(r), :] = acc
        return jnp.where((r & 3) == 3, 0.0, acc)

    x_copies = [pltpu.make_async_copy(ax_hbm, ax_v, x_sem.at[0]), pltpu.make_async_copy(bx_hbm, bx_v, x_sem.at[1])]

    def setup(r, _):
        start_round(r, bwq, None)
        c = lax.broadcasted_iota(jnp.int32, (HD // NR, HD * HG), 0) + r * (HD // NR)
        l = lax.broadcasted_iota(jnp.int32, (HD // NR, HD * HG), 1) >> 3
        e_v[pl.ds(_aligned(r * (HD // NR), HD // NR), HD // NR), :] = jnp.where(c == l, 1.0, 0.0).astype(BF16)

    _loop(NR, setup)
    for copy in x_copies:
        copy.start()
    _loop(NR, lambda r, _: start_round(r, wq, bwq))
    for copy in x_copies:
        copy.wait()
    xa = ax_v[...].astype(F32)
    for b in range(NB):
        for j in range(DM // HD):
            for g in range(NH // HG):
                lat_v[j, pl.ds(g * group + b * HG, HG), :] = jnp.broadcast_to(xa[b:b + 1, j * HD:(j + 1) * HD], (HG, HD))
    xb = bx_v[...].astype(F32)
    xb = jnp.concatenate([xb, xb], axis=0).astype(BF16)

    def b_queries(r, _):
        start_round(r, wuk, wq)
        cols = NH * HD // NR
        w = bwq_v[:, :, pl.ds(_aligned(r * cols, cols), cols)].reshape(DM, cols)
        q = jnp.dot(xb, w, preferred_element_type=F32)
        for k in range(NH // NR):
            qb_v[r * (NH // NR) + k] = q[:, k * HD:(k + 1) * HD]

    wait_all(bwq_v, bwq_sem)
    _loop(NR, b_queries)

    def a_queries(r, acc):
        start_round(r, ckv(0), wuk)
        return up_project(wq_v, r, acc)

    wait_all(wq_v, wq_sem)
    _loop(NR, a_queries, jnp.zeros((2 * group, HD), F32))

    def a_absorb(r, _):
        start_round(r, ckv(1), ckv(0))
        q = head_v[two_groups(r), :].astype(BF16)
        wide = jnp.concatenate([lax.dot_general(q[i * group:(i + 1) * group], weights(wuk_v, r, i), NT,
                                                preferred_element_type=F32) for i in range(2)], axis=0)
        wide = jnp.where(same_head(2 * group), wide, 0.0).astype(BF16)
        lat_v[r & 3, two_groups(r), :] = lax.dot_general(wide, e_v[...], NT, preferred_element_type=F32)

    wait_all(wuk_v, wuk_sem)
    _loop(NR, a_absorb)

    def a_attention(b, _):
        half = NR // 2
        keys = SK // half

        def start(r):
            pl.when(b < 2)(lambda: start_round(r, ckv(b + 2), ckv(b + 1)))
            pl.when(b == 2)(lambda: start_round(r, wuv, ckv(3)))
            pl.when(b == 3)(lambda: start_round(r, k_cache(0), wuv))

        def latents(i):
            return ckv_v[pl.ds(_aligned(b * SK + i * keys, keys), keys), :]

        heads = [pl.ds(_aligned(g * group + b * HG, HG), HG) for g in range(NH // HG)]
        q = jnp.concatenate([jnp.concatenate([lat_v[j, g, :] for g in heads], axis=0)
                             for j in range(DM // HD)], axis=1).astype(BF16)

        def scores(i, m):
            start(i)
            s = lax.dot_general(q, latents(i), NT, preferred_element_type=F32) * scale
            sa_v[i] = s
            return jnp.maximum(m, jnp.max(s, axis=-1, keepdims=True))

        def context(i, carry):
            start(half + i)
            p = jnp.exp(sa_v[i] - m)
            c = jnp.dot(p.astype(BF16), latents(i), preferred_element_type=F32)
            return carry[0] + c, carry[1] + jnp.sum(p, axis=-1, keepdims=True)

        wait_all(ckv_v.at[pl.ds(_aligned(b * SK, SK), SK)], ckv_sem.at[b])
        m = _loop(half, scores, jnp.full((NH, 1), -jnp.inf, F32))
        c, l = _loop(half, context, (jnp.zeros((NH, DM), F32), jnp.zeros((NH, 1), F32)))
        c = c / l
        for j in range(DM // HD):
            for g in range(NH // HG):
                lat_v[j, heads[g], :] = c[g * HG:(g + 1) * HG, j * HD:(j + 1) * HD]

    _loop(NB, a_attention)

    def a_values(r, acc):
        start_round(r, v_cache(0), k_cache(0))
        return up_project(wuv_v, r, acc)

    wait_all(wuv_v, wuv_sem)
    _loop(NR, a_values, jnp.zeros((2 * group, HD), F32))

    keys = SK // NR

    def b_head(h, _):
        q = qb_v[h].astype(BF16)

        def tile(ref, r, b):
            return ref[h & 1, pl.ds(_aligned(b * SK + r * keys, keys), keys), :]

        def scores(r, m):
            pl.when(h + 1 < NH)(lambda: start_round(r, k_cache(h + 1), v_cache(h)))
            pl.when(h + 1 == NH)(lambda: start_round(r, wo, v_cache(NH - 1)))
            row = lax.broadcasted_iota(jnp.int32, (8, keys), 0) % NB
            s = None
            for b in range(NB):
                d = lax.dot_general(q, tile(k_v, r, b), NT, preferred_element_type=F32)
                s = d if s is None else jnp.where(row == b, d, s)
            s = s * scale
            sb_v[r] = s
            return jnp.maximum(m, s)

        def context(r, carry):
            pl.when(h + 1 < NH)(lambda: start_round(r, v_cache(h + 1), k_cache(h + 1)))
            pl.when(h + 1 == NH)(lambda: start_round(r, bwo, wo))
            ctx, l = carry
            p = jnp.exp(sb_v[r] - m)
            for b in range(NB):
                d = jnp.dot(p.astype(BF16), tile(v_v, r, b), preferred_element_type=F32)
                ctx = ctx + jnp.where(row8 == b, d, 0.0)
            return ctx, l + p

        wait_all(k_v.at[h & 1], k_sem.at[h & 1])
        m = jnp.max(_loop(NR, scores, jnp.full((8, keys), -jnp.inf, F32)), axis=-1, keepdims=True)
        wait_all(v_v.at[h & 1], v_sem.at[h & 1])
        ctx, l = _loop(NR, context, (jnp.zeros((8, HD), F32), jnp.zeros((8, keys), F32)))
        cb_v[h] = ctx / jnp.sum(l, axis=-1, keepdims=True)

    _loop(NH, b_head)

    def b_output(i, s):
        return jnp.dot(cb_v[s * (NH // NS) + i].astype(BF16), bwo_v[i, s], preferred_element_type=F32)

    def last_tail(i):
        n = NS * NR - LAG + i
        bwo(0, (n & 7) * NR + (n >> 3), True).start(priority=0)

    def a_output(k, acc):
        for i in range(LAG // NR):
            last_tail(k * (LAG // NR) + i + LAG % NR)
        ctx = head_v[pl.ds(_aligned((k >> 1) * group, group), group), :]
        head = lax.broadcasted_iota(jnp.int32, (group, HD), 0) & (HG - 1)
        lhs = jnp.concatenate([jnp.where(head == (k & 1) * 4 + i, ctx, 0.0) for i in range(4)], axis=1)
        w = wo_v[pl.ds(_aligned(k * DM, DM), DM), :]
        return acc + jnp.dot(lhs.astype(BF16), w, preferred_element_type=F32)

    for i in range(LAG % NR):
        last_tail(i)
    wait_all(wo_v, wo_sem)
    out_a = _loop(NR, a_output, jnp.zeros((group, DM), F32))
    out_ref[:, pl.ds(0, DM)] = jnp.concatenate(
        [jnp.sum(out_a[b * HG:(b + 1) * HG], axis=0, keepdims=True) for b in range(NB)], axis=0).astype(out_ref.dtype)

    def b_outputs(i, acc):
        wait_all(bwo_v.at[i], bwo_sem.at[i])
        for s in range(NS):
            acc = acc + b_output(i, s)
        return acc

    out_b = _loop(3, b_outputs, jnp.zeros((8, DM), F32))
    for streams in LAST:
        for s in streams:
            wait_all(bwo_v.at[3, s], bwo_sem.at[3 + s])
        for s in streams:
            out_b = out_b + b_output(3, s)
    out_ref[:, pl.ds(DM, DM)] = out_b[:NB].astype(out_ref.dtype)


@jax.jit
def pallas_concat_heads__compressed_kv_cla__mha_block_cached__decode_kernel(
    A_x: jax.Array,
    A_c_kv: jax.Array,
    A_w_q: jax.Array,
    A_w_uk: jax.Array,
    A_w_uv: jax.Array,
    A_w_o: jax.Array,
    B_x: jax.Array,
    B_k_cache: jax.Array,
    B_v_cache: jax.Array,
    B_wq: jax.Array,
    B_wo: jax.Array,
):
    assert A_x.shape == (NB, 1, DM) and A_c_kv.shape == (NB, SK, DM) and A_w_q.shape == (DM, NH, HD)
    assert B_x.shape == (NB, 1, DM) and B_k_cache.shape == (NB, NH, SK, HD)
    scratch = [
        pltpu.VMEM((NB, DM), BF16),
        pltpu.VMEM((NB, DM), BF16),
        pltpu.VMEM((NB * SK, DM), BF16),
        pltpu.VMEM((DM, NH, HD), BF16),
        pltpu.VMEM((DM, NH, HD), BF16),
        pltpu.VMEM((DM, NH, HD), BF16),
        pltpu.VMEM((NH * HD, DM), BF16),
        pltpu.VMEM((DM // 8, 8, NH * HD), BF16),
        pltpu.VMEM((NH // NS, NS, HD, DM), BF16),
        pltpu.VMEM((2, NB * SK, HD), BF16),
        pltpu.VMEM((2, NB * SK, HD), BF16),
        pltpu.VMEM((HD, HD * HG), BF16),
        pltpu.VMEM((DM // HD, NB * NH, HD), F32),
        pltpu.VMEM((NB * NH, HD), F32),
        pltpu.VMEM((NR // 2, NH, 2 * SK // NR), F32),
        pltpu.VMEM((NH, 8, HD), F32),
        pltpu.VMEM((NR, 8, SK // NR), F32),
        pltpu.VMEM((NH, 8, HD), F32),
        pltpu.SemaphoreType.DMA((2,)),
        pltpu.SemaphoreType.DMA((5,)),
        pltpu.SemaphoreType.DMA((NB,)),
        pltpu.SemaphoreType.DMA((2,)),
        pltpu.SemaphoreType.DMA((2,)),
        pltpu.SemaphoreType.DMA((3 + NS,)),
    ]
    out = pl.pallas_call(
        _kernel,
        out_shape=jax.ShapeDtypeStruct((NB, 2 * DM), A_x.dtype),
        in_specs=[pl.BlockSpec(memory_space=pl.ANY)] * 11,
        out_specs=pl.BlockSpec(memory_space=pltpu.VMEM),
        scratch_shapes=scratch,
        compiler_params=pltpu.CompilerParams(vmem_limit_bytes=100 * 1024 * 1024, disable_bounds_checks=True, disable_semaphore_checks=NOCHECK),
    )(
        A_x.reshape(NB, DM),
        A_c_kv.reshape(NB * SK, DM),
        A_w_q,
        A_w_uk,
        A_w_uv,
        A_w_o.reshape(NH * HD, DM),
        B_x.reshape(NB, DM),
        B_k_cache.reshape(NB * NH * SK, HD),
        B_v_cache.reshape(NB * NH * SK, HD),
        B_wq,
        B_wo,
    )
    return out.reshape(NB, 1, 2 * DM)
```

```python
import math

import jax
import jax.numpy as jnp
from jax import lax
import jax.experimental.pallas as pl
import jax.experimental.pallas.tpu as pltpu

F32 = jnp.float32
BF16 = jnp.bfloat16
NT = (((1,), (1,)), ((), ()))

NB, NH, SK, HD, DM = 4, 32, 4096, 128, 512
BLOCK = 64 * 1024
NS = 8
NR = 8
LAG = 26
A_SHIFT = 32 * 1024
LEAD = 16 * 1024
LATE = LEAD // (2 * HD)
LAST = ((0, 1, 2, 3), (4, 5), (6, 7))
NOCHECK = True
HG = 8


def _aligned(x, m):
    return x if isinstance(x, int) else pl.multiple_of(x, m)


def _loop(n, body, init=None, lo=0):
    return lax.fori_loop(lo, n, body, init)


def _when(cond, fn):
    if cond is True:
        fn()
    elif cond is not False:
        pl.when(cond)(fn)


def _kernel(ax_hbm, ckv_hbm, wq_hbm, wuk_hbm, wuv_hbm, wo_hbm, bx_hbm, k_hbm, v_hbm, bwq_hbm, bwo_hbm,
            out_ref,
            ax_v, bx_v, ckv_v, wq_v, wuk_v, wuv_v, wo_v, bwq_v, bwo_v, k_v, v_v,
            e_v, lat_v, head_v, sa_v, qb_v, sb_v, cb_v,
            x_sem, bwq_sem, wq_sem, wuk_sem, wuv_sem, wo_sem, ckv_sem, k_sem, v_sem, bwo_sem):
    scale = HD ** -0.5

    def wait_all(dst, sem):
        pltpu.make_async_copy(dst, dst, sem).wait()

    def copy(src, dst, sem, lead):
        pltpu.make_async_copy(src, dst, sem).start(priority=0 if lead else 1)

    def matrix(src, dst, sem, part=0):
        rows = BLOCK // (2 * math.prod(src.shape[1:]))
        shift, split = rows * A_SHIFT // BLOCK, rows * LEAD // BLOCK

        def start(s, r, lead):
            def rows_at(row, size, index=part):
                at = pl.ds(_aligned(row, rows // 4), size)
                copy(src.at[at], dst.at[at], sem.at[index], lead)

            row = ((part * NS + s) * NR + r) * rows - shift
            if s:
                rows_at(*((row, split) if lead else (row + split, rows - split)))
                return
            wrapped, owner = row & (src.shape[0] - 1), (part - jnp.where(r == 0, 1, 0)) & (sem.shape[0] - 1)
            if lead:
                rows_at(wrapped, split, owner)
                return
            pl.when(r > 0)(lambda: rows_at(row + split, rows - split))

            @pl.when(r == 0)
            def _():
                if shift > split:
                    rows_at(wrapped + split, shift - split, owner)
                rows_at(row + shift, rows - shift)

        return start

    def slot(h):
        return jnp.where(h == NH - 1, 2, h & 1)

    def cache(src, dst, sem, h):
        rows = BLOCK // (2 * HD)

        def start(s, r, lead):
            b, key = s // 2, ((s % 2) * NR + r) * rows
            row = (b * NH + h) * SK + key
            if not lead:
                copy(src.at[pl.ds(_aligned(row, rows), rows - LATE)],
                     dst.at[slot(h), b, pl.ds(_aligned(key, rows), rows - LATE)], sem.at[slot(h)], lead)
                return
            row, key, to, index = row - LATE, key - LATE, slot(h), slot(h)
            if s % 2 == 0:
                row, key, to = row & (NB * NH * SK - 1), key & (SK - 1), slot((h - jnp.where(r == 0, 1, 0)) & (NH - 1))
                b, index = row >> 17, to + jnp.where(r == 0, 3, 0)
            copy(src.at[pl.ds(_aligned(row, LATE), LATE)], dst.at[to, b, pl.ds(_aligned(key, LATE), LATE)],
                 sem.at[index], lead)

        return start

    def b_block(s, r, lead):
        return (s * NR + r - 1) & (NS * NR - 1) if lead else s * NR + r

    def bwq(s, r, lead):
        n = b_block(s, r, lead)
        cut = NH * HD - NH * HD * LEAD // BLOCK
        cols = pl.ds(cut, NH * HD - cut) if lead else pl.ds(0, cut)
        copy(bwq_hbm.at[pl.ds(_aligned(n * 8, 8), 8), cols], bwq_v.at[n, :, cols], bwq_sem.at[0], lead)

    def bwo(s, r, lead):
        n = b_block(s, r, lead)
        rows = BLOCK // (2 * DM)
        cut = rows - rows * LEAD // BLOCK
        off, size = (cut, rows - cut) if lead else (0, cut)
        s, i = n >> 3, (n >> 1) & 3
        copy(bwo_hbm.at[pl.ds(_aligned(n * rows + off, 16), size)],
             bwo_v.at[i, s, pl.ds(_aligned((n & 1) * rows + off, 16), size)], bwo_sem.at[jnp.where(i < 3, i, 3 + s)], lead)

    def ckv(b):
        return matrix(ckv_hbm, ckv_v, ckv_sem, b)

    def k_cache(h):
        return cache(k_hbm, k_v, k_sem, h)

    def v_cache(h):
        return cache(v_hbm, v_v, v_sem, h)

    wq, wuk = matrix(wq_hbm, wq_v, wq_sem), matrix(wuk_hbm, wuk_v, wuk_sem)
    wuv, wo = matrix(wuv_hbm, wuv_v, wuv_sem), matrix(wo_hbm, wo_v, wo_sem)

    def start_round(r, unit, previous):
        for streams in (range(LAG % NS), range(LAG % NS, NS)):
            if not streams:
                continue
            back = -((streams[0] - LAG) // NS)

            def start(leads, round_):
                for s in streams:
                    if leads is not None:
                        leads((s - LAG) % NS, round_, True)
                    unit(s, r, False)

            pl.when(r < back)(lambda: start(previous, r + NR - back))
            pl.when(r >= back)(lambda: start(unit, r - back))

    row8 = lax.broadcasted_iota(jnp.int32, (8, HD), 0) & (NB - 1)
    group = NB * HG

    def same_head(rows):
        r = lax.broadcasted_iota(jnp.int32, (rows, HD * HG), 0)
        l = lax.broadcasted_iota(jnp.int32, (rows, HD * HG), 1)
        return (r & (HG - 1)) == (l & (HG - 1))

    def weights(w_ref, r, i):
        c = pl.ds(_aligned((r & 3) * HD, HD), HD)
        h = pl.ds(_aligned(((r >> 2) * 2 + i) * HG, HG), HG)
        return w_ref[c, h, :].reshape(HD * HG, HD)

    def two_groups(r):
        return pl.ds(_aligned((r >> 2) * 2 * group, 2 * group), 2 * group)

    def up_project(w_ref, r, acc):
        wide = jnp.dot(lat_v[r & 3, two_groups(r), :].astype(BF16), e_v[...], preferred_element_type=F32)
        wide = jnp.where(same_head(2 * group), wide, 0.0).astype(BF16)
        acc = acc + jnp.concatenate([jnp.dot(wide[i * group:(i + 1) * group], weights(w_ref, r, i),
                                             preferred_element_type=F32) for i in range(2)], axis=0)
        head_v[two_groups(r), :] = acc
        return jnp.where((r & 3) == 3, 0.0, acc)

    x_copies = [pltpu.make_async_copy(ax_hbm, ax_v, x_sem.at[0]), pltpu.make_async_copy(bx_hbm, bx_v, x_sem.at[1])]

    def setup(r, _):
        start_round(r, bwq, None)
        c = lax.broadcasted_iota(jnp.int32, (HD // NR, HD * HG), 0) + r * (HD // NR)
        l = lax.broadcasted_iota(jnp.int32, (HD // NR, HD * HG), 1) >> 3
        e_v[pl.ds(_aligned(r * (HD // NR), HD // NR), HD // NR), :] = jnp.where(c == l, 1.0, 0.0).astype(BF16)

    _loop(NR, setup)
    for x_copy in x_copies:
        x_copy.start()
    _loop(NR, lambda r, _: start_round(r, wq, bwq))
    for x_copy in x_copies:
        x_copy.wait()
    xa = ax_v[...].astype(F32)
    for b in range(NB):
        for j in range(DM // HD):
            for g in range(NH // HG):
                lat_v[j, pl.ds(g * group + b * HG, HG), :] = jnp.broadcast_to(xa[b:b + 1, j * HD:(j + 1) * HD], (HG, HD))
    xb = bx_v[...].astype(F32)
    xb = jnp.concatenate([xb, xb], axis=0).astype(BF16)

    def b_queries(r, _):
        start_round(r, wuk, wq)
        cols = NH * HD // NR
        w = bwq_v[:, :, pl.ds(_aligned(r * cols, cols), cols)].reshape(DM, cols)
        q = jnp.dot(xb, w, preferred_element_type=F32)
        for k in range(NH // NR):
            qb_v[r * (NH // NR) + k] = q[:, k * HD:(k + 1) * HD]

    wait_all(bwq_v, bwq_sem.at[0])
    _loop(NR, b_queries)

    def a_queries(r, acc):
        start_round(r, ckv(0), wuk)
        return up_project(wq_v, r, acc)

    wait_all(wq_v, wq_sem.at[0])
    _loop(NR, a_queries, jnp.zeros((2 * group, HD), F32))

    def a_absorb(r, _):
        start_round(r, ckv(1), ckv(0))
        q = head_v[two_groups(r), :].astype(BF16)
        wide = jnp.concatenate([lax.dot_general(q[i * group:(i + 1) * group], weights(wuk_v, r, i), NT,
                                                preferred_element_type=F32) for i in range(2)], axis=0)
        wide = jnp.where(same_head(2 * group), wide, 0.0).astype(BF16)
        lat_v[r & 3, two_groups(r), :] = lax.dot_general(wide, e_v[...], NT, preferred_element_type=F32)

    wait_all(wuk_v, wuk_sem.at[0])
    _loop(NR, a_absorb)

    def a_attention(b, _):
        half = NR // 2
        keys = SK // half

        def start(r):
            pl.when(b < 2)(lambda: start_round(r, ckv(b + 2), ckv(b + 1)))
            pl.when(b == 2)(lambda: start_round(r, wuv, ckv(3)))
            pl.when(b == 3)(lambda: start_round(r, k_cache(0), wuv))

        def latents(i):
            return ckv_v[pl.ds(_aligned(b * SK + i * keys, keys), keys), :]

        heads = [pl.ds(_aligned(g * group + b * HG, HG), HG) for g in range(NH // HG)]
        q = jnp.concatenate([jnp.concatenate([lat_v[j, g, :] for g in heads], axis=0)
                             for j in range(DM // HD)], axis=1).astype(BF16)

        def scores(i, m):
            start(i)
            s = lax.dot_general(q, latents(i), NT, preferred_element_type=F32) * scale
            sa_v[i] = s
            return jnp.maximum(m, jnp.max(s, axis=-1, keepdims=True))

        def context(i, carry):
            start(half + i)
            p = jnp.exp(sa_v[i] - m)
            c = jnp.dot(p.astype(BF16), latents(i), preferred_element_type=F32)
            return carry[0] + c, carry[1] + jnp.sum(p, axis=-1, keepdims=True)

        wait_all(ckv_v.at[pl.ds(_aligned(b * SK, SK), SK)], ckv_sem.at[b])
        m = _loop(half, scores, jnp.full((NH, 1), -jnp.inf, F32))
        c, l = _loop(half, context, (jnp.zeros((NH, DM), F32), jnp.zeros((NH, 1), F32)))
        c = c / l
        for j in range(DM // HD):
            for g in range(NH // HG):
                lat_v[j, heads[g], :] = c[g * HG:(g + 1) * HG, j * HD:(j + 1) * HD]

    _loop(NB, a_attention)

    def a_values(r, acc):
        start_round(r, v_cache(0), k_cache(0))
        return up_project(wuv_v, r, acc)

    wait_all(wuv_v, wuv_sem.at[0])
    _loop(NR, a_values, jnp.zeros((2 * group, HD), F32))

    keys = SK // NR

    def b_head(h, _):
        q = qb_v[h].astype(BF16)

        def tile(ref, r, b):
            return ref[slot(h), b, pl.ds(_aligned(r * keys, keys), keys), :]

        def wait_late(ref, sem, r):
            pl.when(r == NR - 1)(lambda: wait_all(ref.at[slot(h), :, pl.ds(SK - LATE, LATE)], sem.at[3 + slot(h)]))

        def scores(r, m):
            pl.when(h + 1 < NH)(lambda: start_round(r, k_cache(h + 1), v_cache(h)))
            pl.when(h + 1 == NH)(lambda: start_round(r, wo, v_cache(NH - 1)))
            wait_late(k_v, k_sem, r)
            row = lax.broadcasted_iota(jnp.int32, (8, keys), 0) & (NB - 1)
            s = None
            for b in range(NB):
                d = lax.dot_general(q, tile(k_v, r, b), NT, preferred_element_type=F32)
                s = d if s is None else jnp.where(row == b, d, s)
            s = s * scale
            sb_v[r] = s
            return jnp.maximum(m, s)

        def context(r, carry):
            pl.when(h + 1 < NH)(lambda: start_round(r, v_cache(h + 1), k_cache(h + 1)))
            pl.when(h + 1 == NH)(lambda: start_round(r, bwo, wo))
            wait_late(v_v, v_sem, r)
            ctx, l = carry
            p = jnp.exp(sb_v[r] - m)
            for b in range(NB):
                d = jnp.dot(p.astype(BF16), tile(v_v, r, b), preferred_element_type=F32)
                ctx = ctx + jnp.where(row8 == b, d, 0.0)
            return ctx, l + p

        wait_all(k_v.at[slot(h), :, pl.ds(0, SK - LATE)], k_sem.at[slot(h)])
        m = jnp.max(_loop(NR, scores, jnp.full((8, keys), -jnp.inf, F32)), axis=-1, keepdims=True)
        wait_all(v_v.at[slot(h), :, pl.ds(0, SK - LATE)], v_sem.at[slot(h)])
        ctx, l = _loop(NR, context, (jnp.zeros((8, HD), F32), jnp.zeros((8, keys), F32)))
        cb_v[h] = ctx / jnp.sum(l, axis=-1, keepdims=True)

    _loop(NH, b_head)

    def b_output(i, s):
        return jnp.dot(cb_v[s * (NH // NS) + i].astype(BF16), bwo_v[i, s], preferred_element_type=F32)

    def last_tail(i):
        n = NS * NR - LAG + i
        bwo(n & 7, n >> 3, True)

    def a_output(k, acc):
        for i in range(LAG // NR):
            last_tail(k * (LAG // NR) + i + LAG % NR)
        ctx = head_v[pl.ds(_aligned((k >> 1) * group, group), group), :]
        head = lax.broadcasted_iota(jnp.int32, (group, HD), 0) & (HG - 1)
        lhs = jnp.concatenate([jnp.where(head == (k & 1) * 4 + i, ctx, 0.0) for i in range(4)], axis=1)
        w = wo_v[pl.ds(_aligned(k * DM, DM), DM), :]
        return acc + jnp.dot(lhs.astype(BF16), w, preferred_element_type=F32)

    for i in range(LAG % NR):
        last_tail(i)
    wait_all(wo_v, wo_sem.at[0])
    out_a = _loop(NR, a_output, jnp.zeros((group, DM), F32))
    out_ref[:, pl.ds(0, DM)] = jnp.concatenate(
        [jnp.sum(out_a[b * HG:(b + 1) * HG], axis=0, keepdims=True) for b in range(NB)], axis=0).astype(out_ref.dtype)

    def b_outputs(i, acc):
        wait_all(bwo_v.at[i], bwo_sem.at[i])
        for s in range(NS):
            acc = acc + b_output(i, s)
        return acc

    out_b = _loop(3, b_outputs, jnp.zeros((8, DM), F32))
    for streams in LAST:
        for s in streams:
            wait_all(bwo_v.at[3, s], bwo_sem.at[3 + s])
        for s in streams:
            out_b = out_b + b_output(3, s)
    out_ref[:, pl.ds(DM, DM)] = out_b[:NB].astype(out_ref.dtype)


@jax.jit
def pallas_concat_heads__compressed_kv_cla__mha_block_cached__decode_kernel(
    A_x: jax.Array,
    A_c_kv: jax.Array,
    A_w_q: jax.Array,
    A_w_uk: jax.Array,
    A_w_uv: jax.Array,
    A_w_o: jax.Array,
    B_x: jax.Array,
    B_k_cache: jax.Array,
    B_v_cache: jax.Array,
    B_wq: jax.Array,
    B_wo: jax.Array,
):
    assert A_x.shape == (NB, 1, DM) and A_c_kv.shape == (NB, SK, DM) and A_w_q.shape == (DM, NH, HD)
    assert B_x.shape == (NB, 1, DM) and B_k_cache.shape == (NB, NH, SK, HD)
    scratch = [
        pltpu.VMEM((NB, DM), BF16),
        pltpu.VMEM((NB, DM), BF16),
        pltpu.VMEM((NB * SK, DM), BF16),
        pltpu.VMEM((DM, NH, HD), BF16),
        pltpu.VMEM((DM, NH, HD), BF16),
        pltpu.VMEM((DM, NH, HD), BF16),
        pltpu.VMEM((NH * HD, DM), BF16),
        pltpu.VMEM((DM // 8, 8, NH * HD), BF16),
        pltpu.VMEM((NH // NS, NS, HD, DM), BF16),
        pltpu.VMEM((3, NB, SK, HD), BF16),
        pltpu.VMEM((3, NB, SK, HD), BF16),
        pltpu.VMEM((HD, HD * HG), BF16),
        pltpu.VMEM((DM // HD, NB * NH, HD), F32),
        pltpu.VMEM((NB * NH, HD), F32),
        pltpu.VMEM((NR // 2, NH, 2 * SK // NR), F32),
        pltpu.VMEM((NH, 8, HD), F32),
        pltpu.VMEM((NR, 8, SK // NR), F32),
        pltpu.VMEM((NH, 8, HD), F32),
        pltpu.SemaphoreType.DMA((2,)),
        *[pltpu.SemaphoreType.DMA((1,))] * 5,
        pltpu.SemaphoreType.DMA((NB,)),
        pltpu.SemaphoreType.DMA((6,)),
        pltpu.SemaphoreType.DMA((6,)),
        pltpu.SemaphoreType.DMA((3 + NS,)),
    ]
    out = pl.pallas_call(
        _kernel,
        out_shape=jax.ShapeDtypeStruct((NB, 2 * DM), A_x.dtype),
        in_specs=[pl.BlockSpec(memory_space=pl.ANY)] * 11,
        out_specs=pl.BlockSpec(memory_space=pltpu.VMEM),
        scratch_shapes=scratch,
        compiler_params=pltpu.CompilerParams(vmem_limit_bytes=100 * 1024 * 1024, disable_bounds_checks=True, disable_semaphore_checks=NOCHECK),
    )(
        A_x.reshape(NB, DM),
        A_c_kv.reshape(NB * SK, DM),
        A_w_q,
        A_w_uk,
        A_w_uv,
        A_w_o.reshape(NH * HD, DM),
        B_x.reshape(NB, DM),
        B_k_cache.reshape(NB * NH * SK, HD),
        B_v_cache.reshape(NB * NH * SK, HD),
        B_wq,
        B_wo,
    )
    return out.reshape(NB, 1, 2 * DM)
```

```python
import math

import jax
import jax.numpy as jnp
from jax import lax
import jax.experimental.pallas as pl
import jax.experimental.pallas.tpu as pltpu

F32 = jnp.float32
BF16 = jnp.bfloat16
NT = (((1,), (1,)), ((), ()))

NB, NH, SK, HD, DM = 4, 32, 4096, 128, 512
BLOCK = 64 * 1024
NS = 8
NR = 8
LAG = 26
A_SHIFT = 32 * 1024
LEAD = 16 * 1024
LATE = LEAD // (2 * HD)
LAST = ((0, 1, 2, 3, 4), (5, 6, 7))
NOCHECK = True
PACE = 0
GAP = 0
RAMP = 0
WHOLE = ()
HG = 8


def _aligned(x, m):
    return x if isinstance(x, int) else pl.multiple_of(x, m)


def _loop(n, body, init=None, lo=0):
    return lax.fori_loop(lo, n, body, init)


def _when(cond, fn):
    if cond is True:
        fn()
    elif cond is not False:
        pl.when(cond)(fn)


def _kernel(ax_hbm, ckv_hbm, wq_hbm, wuk_hbm, wuv_hbm, wo_hbm, bx_hbm, k_hbm, v_hbm, bwq_hbm, bwo_hbm,
            out_ref,
            ax_v, bx_v, ckv_v, wq_v, wuk_v, wuv_v, wo_v, bwq_v, bwo_v, k_v, v_v,
            e_v, lat_v, head_v, sa_v, qb_v, sb_v, cb_v,
            sems):
    scale = HD ** -0.5
    counts = (2, 1, 1, 1, 1, 1, NB, 6, 6, 3 + NS)
    x_sem, bwq_sem, wq_sem, wuk_sem, wuv_sem, wo_sem, ckv_sem, k_sem, v_sem, bwo_sem = (
        sems.at[pl.ds(sum(counts[:i]), n)] for i, n in enumerate(counts))

    def wait_all(dst, sem):
        pltpu.make_async_copy(dst, dst, sem).wait()

    def copy(src, dst, sem, lead):
        pltpu.make_async_copy(src, dst, sem).start(priority=0 if lead else 1)

    def matrix(src, dst, sem, part=0):
        rows = BLOCK // (2 * math.prod(src.shape[1:]))
        shift = rows * A_SHIFT // BLOCK

        def start(s, r, lead):
            row, size, owner = ((part * NS + s) * NR + r) * rows, rows - shift, part
            if lead:
                row, size = row - shift, shift
                if s == 0:
                    row, owner = row & (src.shape[0] - 1), (part - jnp.where(r == 0, 1, 0)) & (sem.shape[0] - 1)
            at = pl.ds(_aligned(row, rows // 4), size)
            copy(src.at[at], dst.at[at], sem.at[owner], lead)

        return start

    def slot(h):
        return jnp.where(h == NH - 1, 2, h & 1)

    def cache(src, dst, sem, h):
        rows = BLOCK // (2 * HD)

        def start(s, r, lead):
            b, key = s // 2, ((s % 2) * NR + r) * rows
            row = (b * NH + h) * SK + key
            if s in WHOLE:
                if not lead:
                    copy(src.at[pl.ds(_aligned(row - LATE, LATE), rows)],
                         dst.at[slot(h), b, pl.ds(_aligned(key - LATE, LATE), rows)], sem.at[slot(h)], lead)
                return
            if not lead:
                copy(src.at[pl.ds(_aligned(row, rows), rows - LATE)],
                     dst.at[slot(h), b, pl.ds(_aligned(key, rows), rows - LATE)], sem.at[slot(h)], lead)
                return
            row, key, to, index = row - LATE, key - LATE, slot(h), slot(h)
            if s % 2 == 0:
                row, key, to = row & (NB * NH * SK - 1), key & (SK - 1), slot((h - jnp.where(r == 0, 1, 0)) & (NH - 1))
                b, index = row >> 17, to + jnp.where(r == 0, 3, 0)
            copy(src.at[pl.ds(_aligned(row, LATE), LATE)], dst.at[to, b, pl.ds(_aligned(key, LATE), LATE)],
                 sem.at[index], lead)

        return start

    def b_block(s, r, lead):
        return (s * NR + r - 1) & (NS * NR - 1) if lead else s * NR + r

    def bwq(s, r, lead):
        n = b_block(s, r, lead)
        cut = NH * HD - NH * HD * LEAD // BLOCK
        cols = pl.ds(cut, NH * HD - cut) if lead else pl.ds(0, cut)
        copy(bwq_hbm.at[pl.ds(_aligned(n * 8, 8), 8), cols], bwq_v.at[n, :, cols], bwq_sem.at[0], lead)

    def bwo(s, r, lead):
        n = b_block(s, r, lead)
        rows = BLOCK // (2 * DM)
        cut = rows - rows * LEAD // BLOCK
        off, size = (cut, rows - cut) if lead else (0, cut)
        s, i = n >> 3, (n >> 1) & 3
        copy(bwo_hbm.at[pl.ds(_aligned(n * rows + off, 16), size)],
             bwo_v.at[i, s, pl.ds(_aligned((n & 1) * rows + off, 16), size)], bwo_sem.at[jnp.where(i < 3, i, 3 + s)], lead)

    def ckv(b):
        return matrix(ckv_hbm, ckv_v, ckv_sem, b)

    def k_cache(h):
        return cache(k_hbm, k_v, k_sem, h)

    def v_cache(h):
        return cache(v_hbm, v_v, v_sem, h)

    wq, wuk = matrix(wq_hbm, wq_v, wq_sem), matrix(wuk_hbm, wuk_v, wuk_sem)
    wuv, wo = matrix(wuv_hbm, wuv_v, wuv_sem), matrix(wo_hbm, wo_v, wo_sem)

    def start_round(r, unit, previous, pace=0):
        def start(first):
            for s in range(NS):
                back, stream = divmod(s - LAG, NS)
                if s >= first:
                    unit(stream, r + back, True)
                elif previous is not None:
                    previous(stream, r + back + NR, True)
                unit(s, r, False)

        pl.when(r < LAG // NS)(lambda: start(NS))
        pl.when(r == LAG // NS)(lambda: start(LAG % NS))
        pl.when(r > LAG // NS)(lambda: start(0))

    row8 = lax.broadcasted_iota(jnp.int32, (8, HD), 0) & (NB - 1)
    group = NB * HG

    def same_head(rows):
        r = lax.broadcasted_iota(jnp.int32, (rows, HD * HG), 0)
        l = lax.broadcasted_iota(jnp.int32, (rows, HD * HG), 1)
        return (r & (HG - 1)) == (l & (HG - 1))

    def weights(w_ref, r, i):
        c = pl.ds(_aligned((r & 3) * HD, HD), HD)
        h = pl.ds(_aligned(((r >> 2) * 2 + i) * HG, HG), HG)
        return w_ref[c, h, :].reshape(HD * HG, HD)

    def two_groups(r):
        return pl.ds(_aligned((r >> 2) * 2 * group, 2 * group), 2 * group)

    def up_project(w_ref, r, acc):
        wide = jnp.dot(lat_v[r & 3, two_groups(r), :].astype(BF16), e_v[...], preferred_element_type=F32)
        wide = jnp.where(same_head(2 * group), wide, 0.0).astype(BF16)
        acc = acc + jnp.concatenate([jnp.dot(wide[i * group:(i + 1) * group], weights(w_ref, r, i),
                                             preferred_element_type=F32) for i in range(2)], axis=0)
        head_v[two_groups(r), :] = acc
        return jnp.where((r & 3) == 3, 0.0, acc)

    x_copies = [pltpu.make_async_copy(ax_hbm, ax_v, x_sem.at[0]), pltpu.make_async_copy(bx_hbm, bx_v, x_sem.at[1])]

    def setup(r, _):
        start_round(r, bwq, None, RAMP)
        c = lax.broadcasted_iota(jnp.int32, (HD // NR, HD * HG), 0) + r * (HD // NR)
        l = lax.broadcasted_iota(jnp.int32, (HD // NR, HD * HG), 1) >> 3
        e_v[pl.ds(_aligned(r * (HD // NR), HD // NR), HD // NR), :] = jnp.where(c == l, 1.0, 0.0).astype(BF16)

    _loop(NR, setup)
    for x_copy in x_copies:
        x_copy.start()
    _loop(NR, lambda r, _: start_round(r, wq, bwq))
    for x_copy in x_copies:
        x_copy.wait()
    xa = ax_v[...].astype(F32)
    for b in range(NB):
        for j in range(DM // HD):
            for g in range(NH // HG):
                lat_v[j, pl.ds(g * group + b * HG, HG), :] = jnp.broadcast_to(xa[b:b + 1, j * HD:(j + 1) * HD], (HG, HD))
    xb = bx_v[...].astype(F32)
    xb = jnp.concatenate([xb, xb], axis=0).astype(BF16)

    def b_queries(r, _):
        start_round(r, wuk, wq)
        cols = NH * HD // NR
        w = bwq_v[:, :, pl.ds(_aligned(r * cols, cols), cols)].reshape(DM, cols)
        q = jnp.dot(xb, w, preferred_element_type=F32)
        for k in range(NH // NR):
            qb_v[r * (NH // NR) + k] = q[:, k * HD:(k + 1) * HD]

    wait_all(bwq_v, bwq_sem.at[0])
    _loop(NR, b_queries)

    def a_queries(r, acc):
        start_round(r, ckv(0), wuk)
        return up_project(wq_v, r, acc)

    wait_all(wq_v, wq_sem.at[0])
    _loop(NR, a_queries, jnp.zeros((2 * group, HD), F32))

    def a_absorb(r, _):
        start_round(r, ckv(1), ckv(0))
        q = head_v[two_groups(r), :].astype(BF16)
        wide = jnp.concatenate([lax.dot_general(q[i * group:(i + 1) * group], weights(wuk_v, r, i), NT,
                                                preferred_element_type=F32) for i in range(2)], axis=0)
        wide = jnp.where(same_head(2 * group), wide, 0.0).astype(BF16)
        lat_v[r & 3, two_groups(r), :] = lax.dot_general(wide, e_v[...], NT, preferred_element_type=F32)

    wait_all(wuk_v, wuk_sem.at[0])
    _loop(NR, a_absorb)

    def a_attention(b, _):
        half = NR // 2
        keys = SK // half

        def start(r):
            pl.when(b < 2)(lambda: start_round(r, ckv(b + 2), ckv(b + 1)))
            pl.when(b == 2)(lambda: start_round(r, wuv, ckv(3)))
            pl.when(b == 3)(lambda: start_round(r, k_cache(0), wuv))

        def latents(i):
            return ckv_v[pl.ds(_aligned(b * SK + i * keys, keys), keys), :]

        heads = [pl.ds(_aligned(g * group + b * HG, HG), HG) for g in range(NH // HG)]
        q = jnp.concatenate([jnp.concatenate([lat_v[j, g, :] for g in heads], axis=0)
                             for j in range(DM // HD)], axis=1).astype(BF16)

        def scores(i, m):
            start(i)
            s = lax.dot_general(q, latents(i), NT, preferred_element_type=F32) * scale
            sa_v[i] = s
            return jnp.maximum(m, jnp.max(s, axis=-1, keepdims=True))

        def context(i, carry):
            start(half + i)
            p = jnp.exp(sa_v[i] - m)
            c = jnp.dot(p.astype(BF16), latents(i), preferred_element_type=F32)
            return carry[0] + c, carry[1] + jnp.sum(p, axis=-1, keepdims=True)

        wait_all(ckv_v.at[pl.ds(_aligned(b * SK, SK), SK)], ckv_sem.at[b])
        m = _loop(half, scores, jnp.full((NH, 1), -jnp.inf, F32))
        c, l = _loop(half, context, (jnp.zeros((NH, DM), F32), jnp.zeros((NH, 1), F32)))
        c = c / l
        for j in range(DM // HD):
            for g in range(NH // HG):
                lat_v[j, heads[g], :] = c[g * HG:(g + 1) * HG, j * HD:(j + 1) * HD]

    _loop(NB, a_attention)

    def a_values(r, acc):
        start_round(r, v_cache(0), k_cache(0))
        return up_project(wuv_v, r, acc)

    wait_all(wuv_v, wuv_sem.at[0])
    _loop(NR, a_values, jnp.zeros((2 * group, HD), F32))

    keys = SK // NR

    def b_head(h, _):
        q = qb_v[h].astype(BF16)

        def tile(ref, r, b):
            return ref[slot(h), b, pl.ds(_aligned(r * keys, keys), keys), :]

        def wait_late(ref, sem, r):
            pl.when(r == NR - 1)(lambda: wait_all(ref.at[slot(h), :, pl.ds(SK - LATE, LATE)], sem.at[3 + slot(h)]))

        def scores(r, m):
            pl.when(h + 1 < NH)(lambda: start_round(r, k_cache(h + 1), v_cache(h)))
            pl.when(h + 1 == NH)(lambda: start_round(r, wo, v_cache(NH - 1)))
            wait_late(k_v, k_sem, r)
            row = lax.broadcasted_iota(jnp.int32, (8, keys), 0) & (NB - 1)
            s = None
            for b in range(NB):
                d = lax.dot_general(q, tile(k_v, r, b), NT, preferred_element_type=F32)
                s = d if s is None else jnp.where(row == b, d, s)
            s = s * scale
            sb_v[r] = s
            return jnp.maximum(m, s)

        def context(r, carry):
            pl.when(h + 1 < NH)(lambda: start_round(r, v_cache(h + 1), k_cache(h + 1)))
            pl.when(h + 1 == NH)(lambda: start_round(r, bwo, wo))
            wait_late(v_v, v_sem, r)
            ctx, l = carry
            p = jnp.exp(sb_v[r] - m)
            for b in range(NB):
                d = jnp.dot(p.astype(BF16), tile(v_v, r, b), preferred_element_type=F32)
                ctx = ctx + jnp.where(row8 == b, d, 0.0)
            return ctx, l + p

        wait_all(k_v.at[slot(h), :, pl.ds(0, SK - LATE)], k_sem.at[slot(h)])
        m = jnp.max(_loop(NR, scores, jnp.full((8, keys), -jnp.inf, F32)), axis=-1, keepdims=True)
        wait_all(v_v.at[slot(h), :, pl.ds(0, SK - LATE)], v_sem.at[slot(h)])
        ctx, l = _loop(NR, context, (jnp.zeros((8, HD), F32), jnp.zeros((8, keys), F32)))
        cb_v[h] = ctx / jnp.sum(l, axis=-1, keepdims=True)

    _loop(NH, b_head)

    def b_output(i, s):
        return jnp.dot(cb_v[s * (NH // NS) + i].astype(BF16), bwo_v[i, s], preferred_element_type=F32)

    def last_tail(i):
        n = NS * NR - LAG + i
        bwo(n & 7, n >> 3, True)

    def a_output(k, acc):
        for i in range(LAG // NR if not PACE else 0):
            last_tail(k * (LAG // NR) + i + LAG % NR)
            if GAP:
                pl.delay(GAP)
        ctx = head_v[pl.ds(_aligned((k >> 1) * group, group), group), :]
        head = lax.broadcasted_iota(jnp.int32, (group, HD), 0) & (HG - 1)
        lhs = jnp.concatenate([jnp.where(head == (k & 1) * 4 + i, ctx, 0.0) for i in range(4)], axis=1)
        w = wo_v[pl.ds(_aligned(k * DM, DM), DM), :]
        return acc + jnp.dot(lhs.astype(BF16), w, preferred_element_type=F32)

    def paced(i, _):
        last_tail(i)
        pl.delay(PACE)

    if PACE:
        _loop(LAG, paced)
    else:
        for i in range(LAG % NR):
            last_tail(i)
    wait_all(wo_v, wo_sem.at[0])
    out_a = _loop(NR, a_output, jnp.zeros((group, DM), F32))
    out_ref[:, pl.ds(0, DM)] = jnp.concatenate(
        [jnp.sum(out_a[b * HG:(b + 1) * HG], axis=0, keepdims=True) for b in range(NB)], axis=0).astype(out_ref.dtype)

    def b_outputs(i, acc):
        wait_all(bwo_v.at[i], bwo_sem.at[i])
        for s in range(NS):
            acc = acc + b_output(i, s)
        return acc

    out_b = _loop(3, b_outputs, jnp.zeros((8, DM), F32))
    for streams in LAST:
        for s in streams:
            wait_all(bwo_v.at[3, s], bwo_sem.at[3 + s])
        for s in streams:
            out_b = out_b + b_output(3, s)
    out_ref[:, pl.ds(DM, DM)] = out_b[:NB].astype(out_ref.dtype)


@jax.jit
def pallas_concat_heads__compressed_kv_cla__mha_block_cached__decode_kernel(
    A_x: jax.Array,
    A_c_kv: jax.Array,
    A_w_q: jax.Array,
    A_w_uk: jax.Array,
    A_w_uv: jax.Array,
    A_w_o: jax.Array,
    B_x: jax.Array,
    B_k_cache: jax.Array,
    B_v_cache: jax.Array,
    B_wq: jax.Array,
    B_wo: jax.Array,
):
    assert A_x.shape == (NB, 1, DM) and A_c_kv.shape == (NB, SK, DM) and A_w_q.shape == (DM, NH, HD)
    assert B_x.shape == (NB, 1, DM) and B_k_cache.shape == (NB, NH, SK, HD)
    scratch = [
        pltpu.VMEM((NB, DM), BF16),
        pltpu.VMEM((NB, DM), BF16),
        pltpu.VMEM((NB * SK, DM), BF16),
        pltpu.VMEM((DM, NH, HD), BF16),
        pltpu.VMEM((DM, NH, HD), BF16),
        pltpu.VMEM((DM, NH, HD), BF16),
        pltpu.VMEM((NH * HD, DM), BF16),
        pltpu.VMEM((DM // 8, 8, NH * HD), BF16),
        pltpu.VMEM((NH // NS, NS, HD, DM), BF16),
        pltpu.VMEM((3, NB, SK, HD), BF16),
        pltpu.VMEM((3, NB, SK, HD), BF16),
        pltpu.VMEM((HD, HD * HG), BF16),
        pltpu.VMEM((DM // HD, NB * NH, HD), F32),
        pltpu.VMEM((NB * NH, HD), F32),
        pltpu.VMEM((NR // 2, NH, 2 * SK // NR), F32),
        pltpu.VMEM((NH, 8, HD), F32),
        pltpu.VMEM((NR, 8, SK // NR), F32),
        pltpu.VMEM((NH, 8, HD), F32),
        pltpu.SemaphoreType.DMA((34,)),
    ]
    out = pl.pallas_call(
        _kernel,
        out_shape=jax.ShapeDtypeStruct((NB, 2 * DM), A_x.dtype),
        in_specs=[pl.BlockSpec(memory_space=pl.ANY)] * 11,
        out_specs=pl.BlockSpec(memory_space=pltpu.VMEM),
        scratch_shapes=scratch,
        compiler_params=pltpu.CompilerParams(vmem_limit_bytes=100 * 1024 * 1024, disable_bounds_checks=True, disable_semaphore_checks=NOCHECK),
    )(
        A_x.reshape(NB, DM),
        A_c_kv.reshape(NB * SK, DM),
        A_w_q,
        A_w_uk,
        A_w_uv,
        A_w_o.reshape(NH * HD, DM),
        B_x.reshape(NB, DM),
        B_k_cache.reshape(NB * NH * SK, HD),
        B_v_cache.reshape(NB * NH * SK, HD),
        B_wq,
        B_wo,
    )
    return out.reshape(NB, 1, 2 * DM)
```

```python
import math

import jax
import jax.numpy as jnp
from jax import lax
import jax.experimental.pallas as pl
import jax.experimental.pallas.tpu as pltpu

F32 = jnp.float32
BF16 = jnp.bfloat16
NT = (((1,), (1,)), ((), ()))

NB, NH, SK, HD, DM = 4, 32, 4096, 128, 512
HG = 8
GROUP = NB * HG
BLOCK = 64 * 1024
NS = 8
NR = 8
LAG = 26
A_LEAD = 32 * 1024
B_LEAD = 16 * 1024
LATE = B_LEAD // (2 * HD)
SLOTS = 3
SEMS = (2, 1, 1, 1, 1, 1, NB, 2 * SLOTS, 2 * SLOTS, NH // NS - 1 + NS)


def _aligned(x, m):
    return x if isinstance(x, int) else pl.multiple_of(x, m)


def _tile(i, size):
    return pl.ds(_aligned(i * size, size), size)


def _loop(n, body, init=None):
    return lax.fori_loop(0, n, body, init)


def _kernel(ax_hbm, ckv_hbm, wq_hbm, wuk_hbm, wuv_hbm, wo_hbm, bx_hbm, k_hbm, v_hbm, bwq_hbm, bwo_hbm,
            out_ref,
            ax_v, bx_v, ckv_v, wq_v, wuk_v, wuv_v, wo_v, bwq_v, bwo_v, k_v, v_v,
            e_v, lat_v, head_v, sa_v, qb_v, sb_v, cb_v, sems):
    scale = HD ** -0.5
    x_sem, bwq_sem, wq_sem, wuk_sem, wuv_sem, wo_sem, ckv_sem, k_sem, v_sem, bwo_sem = (
        sems.at[pl.ds(sum(SEMS[:i]), n)] for i, n in enumerate(SEMS))

    def copy(src, dst, sem, lead):
        pltpu.make_async_copy(src, dst, sem).start(priority=0 if lead else 1)

    def wait_all(dst, sem):
        pltpu.make_async_copy(dst, dst, sem).wait()

    def matrix(src, dst, sem, part=0):
        rows = BLOCK // (2 * math.prod(src.shape[1:]))
        shift = rows * A_LEAD // BLOCK

        def unit(s, r, lead):
            row, size, owner = ((part * NS + s) * NR + r) * rows, rows - shift, part
            if lead:
                row, size = row - shift, shift
                if s == 0:
                    row = row & (src.shape[0] - 1)
                    owner = (part - jnp.where(r == 0, 1, 0)) & (sem.shape[0] - 1)
            at = pl.ds(_aligned(row, math.gcd(rows, shift)), size)
            copy(src.at[at], dst.at[at], sem.at[owner], lead)

        return unit

    def slot(h):
        return jnp.where(h == NH - 1, SLOTS - 1, h & 1)

    def cache(src, dst, sem, h):
        rows = BLOCK // (2 * HD)

        def unit(s, r, lead):
            b, key = s // 2, (s % 2 * NR + r) * rows
            row, size, to, owner = (b * NH + h) * SK + key, rows - LATE, slot(h), slot(h)
            if lead:
                row, key, size = row - LATE, key - LATE, LATE
                if s % 2 == 0:
                    row, key = row & (NB * NH * SK - 1), key & (SK - 1)
                    b = row >> (NH * SK).bit_length() - 1
                    to = slot((h - jnp.where(r == 0, 1, 0)) & (NH - 1))
                    owner = to + jnp.where(r == 0, SLOTS, 0)
            align = math.gcd(rows, LATE)
            copy(src.at[pl.ds(_aligned(row, align), size)], dst.at[to, b, pl.ds(_aligned(key, align), size)],
                 sem.at[owner], lead)

        return unit

    def b_piece(s, r, lead, width):
        cut = width - width * B_LEAD // BLOCK
        if lead:
            return (s * NR + r - 1) & (NS * NR - 1), cut, width - cut
        return s * NR + r, 0, cut

    def bwq(s, r, lead):
        n, off, size = b_piece(s, r, lead, NH * HD)
        copy(bwq_hbm.at[_tile(n, 8), pl.ds(off, size)], bwq_v.at[n, :, pl.ds(off, size)], bwq_sem.at[0], lead)

    def bwo(s, r, lead):
        rows = BLOCK // (2 * DM)
        n, off, size = b_piece(s, r, lead, rows)
        s, i = n >> 3, (n >> 1) & 3
        copy(bwo_hbm.at[pl.ds(_aligned(n * rows + off, 16), size)],
             bwo_v.at[i, s, pl.ds(_aligned((n & 1) * rows + off, 16), size)],
             bwo_sem.at[jnp.where(i < 3, i, 3 + s)], lead)

    def ckv(b):
        return matrix(ckv_hbm, ckv_v, ckv_sem, b)

    def k_cache(h):
        return cache(k_hbm, k_v, k_sem, h)

    def v_cache(h):
        return cache(v_hbm, v_v, v_sem, h)

    wq, wuk = matrix(wq_hbm, wq_v, wq_sem), matrix(wuk_hbm, wuk_v, wuk_sem)
    wuv, wo = matrix(wuv_hbm, wuv_v, wuv_sem), matrix(wo_hbm, wo_v, wo_sem)

    def start_round(r, unit, previous):
        def start(first):
            for s in range(NS):
                back, stream = divmod(s - LAG, NS)
                if s >= first:
                    unit(stream, r + back, True)
                elif previous is not None:
                    previous(stream, r + back + NR, True)
                unit(s, r, False)

        pl.when(r < LAG // NS)(lambda: start(NS))
        pl.when(r == LAG // NS)(lambda: start(LAG % NS))
        pl.when(r > LAG // NS)(lambda: start(0))

    def same_head():
        row = lax.broadcasted_iota(jnp.int32, (2 * GROUP, HD * HG), 0)
        col = lax.broadcasted_iota(jnp.int32, (2 * GROUP, HD * HG), 1)
        return (row & (HG - 1)) == (col & (HG - 1))

    def weights(w_ref, r, i):
        return w_ref[_tile(r & 3, HD), _tile((r >> 2) * 2 + i, HG), :].reshape(HD * HG, HD)

    def up_project(w_ref, r, acc):
        rows = _tile(r >> 2, 2 * GROUP)
        wide = jnp.dot(lat_v[r & 3, rows, :].astype(BF16), e_v[...], preferred_element_type=F32)
        wide = jnp.where(same_head(), wide, 0.0).astype(BF16)
        acc = acc + jnp.concatenate([jnp.dot(wide[i * GROUP:(i + 1) * GROUP], weights(w_ref, r, i),
                                             preferred_element_type=F32) for i in range(2)], axis=0)
        head_v[rows, :] = acc
        return jnp.where((r & 3) == 3, 0.0, acc)

    def setup(r, _):
        start_round(r, bwq, None)
        c = lax.broadcasted_iota(jnp.int32, (HD // NR, HD * HG), 0) + r * (HD // NR)
        col = lax.broadcasted_iota(jnp.int32, (HD // NR, HD * HG), 1)
        e_v[_tile(r, HD // NR), :] = jnp.where(c == col >> HG.bit_length() - 1, 1.0, 0.0).astype(BF16)

    _loop(NR, setup)
    x_copies = [pltpu.make_async_copy(ax_hbm, ax_v, x_sem.at[0]), pltpu.make_async_copy(bx_hbm, bx_v, x_sem.at[1])]
    for x_copy in x_copies:
        x_copy.start()
    _loop(NR, lambda r, _: start_round(r, wq, bwq))
    for x_copy in x_copies:
        x_copy.wait()
    xa = ax_v[...].astype(F32)
    for b in range(NB):
        for j in range(DM // HD):
            for g in range(NH // HG):
                lat_v[j, _tile(g * NB + b, HG), :] = jnp.broadcast_to(xa[b:b + 1, j * HD:(j + 1) * HD], (HG, HD))
    xb = bx_v[...].astype(F32)
    xb = jnp.concatenate([xb, xb], axis=0).astype(BF16)

    def b_queries(r, _):
        start_round(r, wuk, wq)
        cols = NH * HD // NR
        q = jnp.dot(xb, bwq_v[:, :, _tile(r, cols)].reshape(DM, cols), preferred_element_type=F32)
        for i in range(NH // NR):
            qb_v[r * (NH // NR) + i] = q[:, i * HD:(i + 1) * HD]

    wait_all(bwq_v, bwq_sem.at[0])
    _loop(NR, b_queries)

    def a_queries(r, acc):
        start_round(r, ckv(0), wuk)
        return up_project(wq_v, r, acc)

    wait_all(wq_v, wq_sem.at[0])
    _loop(NR, a_queries, jnp.zeros((2 * GROUP, HD), F32))

    def a_absorb(r, _):
        start_round(r, ckv(1), ckv(0))
        rows = _tile(r >> 2, 2 * GROUP)
        q = head_v[rows, :].astype(BF16)
        wide = jnp.concatenate([lax.dot_general(q[i * GROUP:(i + 1) * GROUP], weights(wuk_v, r, i), NT,
                                                preferred_element_type=F32) for i in range(2)], axis=0)
        wide = jnp.where(same_head(), wide, 0.0).astype(BF16)
        lat_v[r & 3, rows, :] = lax.dot_general(wide, e_v[...], NT, preferred_element_type=F32)

    wait_all(wuk_v, wuk_sem.at[0])
    _loop(NR, a_absorb)

    def a_attention(b, _):
        steps = NR // 2

        def start(r):
            pl.when(b < 2)(lambda: start_round(r, ckv(b + 2), ckv(b + 1)))
            pl.when(b == 2)(lambda: start_round(r, wuv, ckv(3)))
            pl.when(b == 3)(lambda: start_round(r, k_cache(0), wuv))

        def latents(i):
            return ckv_v[_tile(b * steps + i, SK // steps), :]

        heads = [_tile(g * NB + b, HG) for g in range(NH // HG)]
        q = jnp.concatenate([jnp.concatenate([lat_v[j, rows, :] for rows in heads], axis=0)
                             for j in range(DM // HD)], axis=1).astype(BF16)

        def scores(i, m):
            start(i)
            s = lax.dot_general(q, latents(i), NT, preferred_element_type=F32) * scale
            sa_v[i] = s
            return jnp.maximum(m, jnp.max(s, axis=-1, keepdims=True))

        def context(i, carry):
            start(steps + i)
            p = jnp.exp(sa_v[i] - m)
            c = jnp.dot(p.astype(BF16), latents(i), preferred_element_type=F32)
            return carry[0] + c, carry[1] + jnp.sum(p, axis=-1, keepdims=True)

        wait_all(ckv_v.at[_tile(b, SK)], ckv_sem.at[b])
        m = _loop(steps, scores, jnp.full((NH, 1), -jnp.inf, F32))
        c, l = _loop(steps, context, (jnp.zeros((NH, DM), F32), jnp.zeros((NH, 1), F32)))
        c = c / l
        for j in range(DM // HD):
            for g, rows in enumerate(heads):
                lat_v[j, rows, :] = c[g * HG:(g + 1) * HG, j * HD:(j + 1) * HD]

    _loop(NB, a_attention)

    def a_values(r, acc):
        start_round(r, v_cache(0), k_cache(0))
        return up_project(wuv_v, r, acc)

    wait_all(wuv_v, wuv_sem.at[0])
    _loop(NR, a_values, jnp.zeros((2 * GROUP, HD), F32))

    def b_head(h, _):
        step = SK // NR
        q = qb_v[h].astype(BF16)

        def batch(width):
            return lax.broadcasted_iota(jnp.int32, (2 * NB, width), 0) & (NB - 1)

        def wait_bulk(ref, sem):
            wait_all(ref.at[slot(h), :, pl.ds(0, SK - LATE)], sem.at[slot(h)])

        def wait_late(ref, sem, r):
            pl.when(r == NR - 1)(lambda: wait_all(ref.at[slot(h), :, pl.ds(SK - LATE, LATE)], sem.at[SLOTS + slot(h)]))

        def scores(r, m):
            pl.when(h + 1 < NH)(lambda: start_round(r, k_cache(h + 1), v_cache(h)))
            pl.when(h + 1 == NH)(lambda: start_round(r, wo, v_cache(NH - 1)))
            wait_late(k_v, k_sem, r)
            s = None
            for b in range(NB):
                d = lax.dot_general(q, k_v[slot(h), b, _tile(r, step), :], NT, preferred_element_type=F32)
                s = d if s is None else jnp.where(batch(step) == b, d, s)
            s = s * scale
            sb_v[r] = s
            return jnp.maximum(m, s)

        def context(r, carry):
            pl.when(h + 1 < NH)(lambda: start_round(r, v_cache(h + 1), k_cache(h + 1)))
            pl.when(h + 1 == NH)(lambda: start_round(r, bwo, wo))
            wait_late(v_v, v_sem, r)
            ctx, l = carry
            p = jnp.exp(sb_v[r] - m)
            for b in range(NB):
                d = jnp.dot(p.astype(BF16), v_v[slot(h), b, _tile(r, step), :], preferred_element_type=F32)
                ctx = ctx + jnp.where(batch(HD) == b, d, 0.0)
            return ctx, l + p

        wait_bulk(k_v, k_sem)
        m = jnp.max(_loop(NR, scores, jnp.full((2 * NB, step), -jnp.inf, F32)), axis=-1, keepdims=True)
        wait_bulk(v_v, v_sem)
        ctx, l = _loop(NR, context, (jnp.zeros((2 * NB, HD), F32), jnp.zeros((2 * NB, step), F32)))
        cb_v[h] = ctx / jnp.sum(l, axis=-1, keepdims=True)

    _loop(NH, b_head)
    for n in range(NS * NR - LAG, NS * NR):
        bwo(n % NS, n // NS, True)

    def a_output(i, acc):
        heads = NH // NR
        ctx = head_v[_tile(i >> 1, GROUP), :]
        head = lax.broadcasted_iota(jnp.int32, (GROUP, HD), 0) & (HG - 1)
        lhs = jnp.concatenate([jnp.where(head == (i & 1) * heads + j, ctx, 0.0) for j in range(heads)], axis=1)
        return acc + jnp.dot(lhs.astype(BF16), wo_v[_tile(i, heads * HD), :], preferred_element_type=F32)

    wait_all(wo_v, wo_sem.at[0])
    out_a = _loop(NR, a_output, jnp.zeros((GROUP, DM), F32))
    out_a = [jnp.sum(out_a[b * HG:(b + 1) * HG], axis=0, keepdims=True) for b in range(NB)]
    out_ref[:, pl.ds(0, DM)] = jnp.concatenate(out_a, axis=0).astype(out_ref.dtype)

    def b_output(i, streams, acc):
        for s in streams:
            acc = acc + jnp.dot(cb_v[s * (NH // NS) + i].astype(BF16), bwo_v[i, s], preferred_element_type=F32)
        return acc

    def b_outputs(i, acc):
        wait_all(bwo_v.at[i], bwo_sem.at[i])
        return b_output(i, range(NS), acc)

    out_b = _loop(3, b_outputs, jnp.zeros((2 * NB, DM), F32))
    for streams in (range(NS // 2), range(NS // 2, NS)):
        for s in streams:
            wait_all(bwo_v.at[3, s], bwo_sem.at[3 + s])
        out_b = b_output(3, streams, out_b)
    out_ref[:, pl.ds(DM, DM)] = out_b[:NB].astype(out_ref.dtype)


@jax.jit
def pallas_concat_heads__compressed_kv_cla__mha_block_cached__decode_kernel(
    A_x: jax.Array,
    A_c_kv: jax.Array,
    A_w_q: jax.Array,
    A_w_uk: jax.Array,
    A_w_uv: jax.Array,
    A_w_o: jax.Array,
    B_x: jax.Array,
    B_k_cache: jax.Array,
    B_v_cache: jax.Array,
    B_wq: jax.Array,
    B_wo: jax.Array,
):
    assert A_x.shape == (NB, 1, DM) and A_c_kv.shape == (NB, SK, DM) and A_w_q.shape == (DM, NH, HD)
    assert B_x.shape == (NB, 1, DM) and B_k_cache.shape == (NB, NH, SK, HD)
    scratch = [
        pltpu.VMEM((NB, DM), BF16),
        pltpu.VMEM((NB, DM), BF16),
        pltpu.VMEM((NB * SK, DM), BF16),
        pltpu.VMEM((DM, NH, HD), BF16),
        pltpu.VMEM((DM, NH, HD), BF16),
        pltpu.VMEM((DM, NH, HD), BF16),
        pltpu.VMEM((NH * HD, DM), BF16),
        pltpu.VMEM((DM // 8, 8, NH * HD), BF16),
        pltpu.VMEM((NH // NS, NS, HD, DM), BF16),
        pltpu.VMEM((SLOTS, NB, SK, HD), BF16),
        pltpu.VMEM((SLOTS, NB, SK, HD), BF16),
        pltpu.VMEM((HD, HD * HG), BF16),
        pltpu.VMEM((DM // HD, NB * NH, HD), F32),
        pltpu.VMEM((NB * NH, HD), F32),
        pltpu.VMEM((NR // 2, NH, 2 * SK // NR), F32),
        pltpu.VMEM((NH, 2 * NB, HD), F32),
        pltpu.VMEM((NR, 2 * NB, SK // NR), F32),
        pltpu.VMEM((NH, 2 * NB, HD), F32),
        pltpu.SemaphoreType.DMA((sum(SEMS),)),
    ]
    out = pl.pallas_call(
        _kernel,
        out_shape=jax.ShapeDtypeStruct((NB, 2 * DM), A_x.dtype),
        in_specs=[pl.BlockSpec(memory_space=pl.ANY)] * 11,
        out_specs=pl.BlockSpec(memory_space=pltpu.VMEM),
        scratch_shapes=scratch,
        compiler_params=pltpu.CompilerParams(
            vmem_limit_bytes=100 * 1024 * 1024, disable_bounds_checks=True, disable_semaphore_checks=True),
    )(
        A_x.reshape(NB, DM),
        A_c_kv.reshape(NB * SK, DM),
        A_w_q,
        A_w_uk,
        A_w_uv,
        A_w_o.reshape(NH * HD, DM),
        B_x.reshape(NB, DM),
        B_k_cache.reshape(NB * NH * SK, HD),
        B_v_cache.reshape(NB * NH * SK, HD),
        B_wq,
        B_wo,
    )
    return out.reshape(NB, 1, 2 * DM)
```

```python
import math

import jax
import jax.numpy as jnp
from jax import lax
import jax.experimental.pallas as pl
import jax.experimental.pallas.tpu as pltpu

F32 = jnp.float32
BF16 = jnp.bfloat16
NT = (((1,), (1,)), ((), ()))

NB, NH, SK, HD, DM = 4, 32, 4096, 128, 512
HG = 8
GROUP = NB * HG
BLOCK = 64 * 1024
NS = 8
NR = 8
LAG = 26
A_LEAD = 32 * 1024
B_LEAD = 16 * 1024
LATE = B_LEAD // (2 * HD)
SLOTS = 3
SEMS = (2, 1, 1, 1, 1, 1, NB, 2 * SLOTS, 2 * SLOTS, NH // NS - 1 + NS)


def _aligned(x, m):
    return x if isinstance(x, int) else pl.multiple_of(x, m)


def _tile(i, size):
    return pl.ds(_aligned(i * size, size), size)


def _loop(n, body, init=None):
    return lax.fori_loop(0, n, body, init)


def _kernel(*refs):
    pl.run_scoped(lambda sems: _body(*refs, sems), pltpu.SemaphoreType.DMA((sum(SEMS),)))


def _body(ax_hbm, ckv_hbm, wq_hbm, wuk_hbm, wuv_hbm, wo_hbm, bx_hbm, k_hbm, v_hbm, bwq_hbm, bwo_hbm,
          out_ref,
          ax_v, bx_v, ckv_v, wq_v, wuk_v, wuv_v, wo_v, bwq_v, bwo_v, k_v, v_v,
          e_v, lat_v, head_v, sa_v, qb_v, sb_v, cb_v, sems):
    scale = HD ** -0.5
    x_sem, bwq_sem, wq_sem, wuk_sem, wuv_sem, wo_sem, ckv_sem, k_sem, v_sem, bwo_sem = (
        sems.at[pl.ds(sum(SEMS[:i]), n)] for i, n in enumerate(SEMS))

    def copy(src, dst, sem, lead):
        pltpu.make_async_copy(src, dst, sem).start(priority=0 if lead else 1)

    def wait_all(dst, sem):
        pltpu.make_async_copy(dst, dst, sem).wait()

    def matrix(src, dst, sem, part=0):
        rows = BLOCK // (2 * math.prod(src.shape[1:]))
        shift = rows * A_LEAD // BLOCK

        def unit(s, r, lead):
            row, size, owner = ((part * NS + s) * NR + r) * rows, rows - shift, part
            if lead:
                row, size = row - shift, shift
                if s == 0:
                    row = row & (src.shape[0] - 1)
                    owner = (part - jnp.where(r == 0, 1, 0)) & (sem.shape[0] - 1)
            at = pl.ds(_aligned(row, math.gcd(rows, shift)), size)
            copy(src.at[at], dst.at[at], sem.at[owner], lead)

        return unit

    def slot(h):
        return jnp.where(h == NH - 1, SLOTS - 1, h & 1)

    def cache(src, dst, sem, h):
        rows = BLOCK // (2 * HD)

        def unit(s, r, lead):
            b, key = s // 2, (s % 2 * NR + r) * rows
            row, size, to, owner = (b * NH + h) * SK + key, rows - LATE, slot(h), slot(h)
            if lead:
                row, key, size = row - LATE, key - LATE, LATE
                if s % 2 == 0:
                    row, key = row & (NB * NH * SK - 1), key & (SK - 1)
                    b = row >> (NH * SK).bit_length() - 1
                    to = slot((h - jnp.where(r == 0, 1, 0)) & (NH - 1))
                    owner = to + jnp.where(r == 0, SLOTS, 0)
            align = math.gcd(rows, LATE)
            copy(src.at[pl.ds(_aligned(row, align), size)], dst.at[to, b, pl.ds(_aligned(key, align), size)],
                 sem.at[owner], lead)

        return unit

    def b_piece(s, r, lead, width):
        cut = width - width * B_LEAD // BLOCK
        if lead:
            return (s * NR + r - 1) & (NS * NR - 1), cut, width - cut
        return s * NR + r, 0, cut

    def bwq(s, r, lead):
        n, off, size = b_piece(s, r, lead, NH * HD)
        copy(bwq_hbm.at[_tile(n, 8), pl.ds(off, size)], bwq_v.at[n, :, pl.ds(off, size)], bwq_sem.at[0], lead)

    def bwo(s, r, lead):
        rows = BLOCK // (2 * DM)
        n, off, size = b_piece(s, r, lead, rows)
        s, i = n >> 3, (n >> 1) & 3
        copy(bwo_hbm.at[pl.ds(_aligned(n * rows + off, 16), size)],
             bwo_v.at[i, s, pl.ds(_aligned((n & 1) * rows + off, 16), size)],
             bwo_sem.at[jnp.where(i < 3, i, 3 + s)], lead)

    def ckv(b):
        return matrix(ckv_hbm, ckv_v, ckv_sem, b)

    def k_cache(h):
        return cache(k_hbm, k_v, k_sem, h)

    def v_cache(h):
        return cache(v_hbm, v_v, v_sem, h)

    wq, wuk = matrix(wq_hbm, wq_v, wq_sem), matrix(wuk_hbm, wuk_v, wuk_sem)
    wuv, wo = matrix(wuv_hbm, wuv_v, wuv_sem), matrix(wo_hbm, wo_v, wo_sem)

    def start_round(r, unit, previous):
        def start(first):
            for s in range(NS):
                back, stream = divmod(s - LAG, NS)
                if s >= first:
                    unit(stream, r + back, True)
                elif previous is not None:
                    previous(stream, r + back + NR, True)
                unit(s, r, False)

        pl.when(r < LAG // NS)(lambda: start(NS))
        pl.when(r == LAG // NS)(lambda: start(LAG % NS))
        pl.when(r > LAG // NS)(lambda: start(0))

    def same_head():
        row = lax.broadcasted_iota(jnp.int32, (2 * GROUP, HD * HG), 0)
        col = lax.broadcasted_iota(jnp.int32, (2 * GROUP, HD * HG), 1)
        return (row & (HG - 1)) == (col & (HG - 1))

    def weights(w_ref, r, i):
        return w_ref[_tile(r & 3, HD), _tile((r >> 2) * 2 + i, HG), :].reshape(HD * HG, HD)

    def up_project(w_ref, r, acc):
        rows = _tile(r >> 2, 2 * GROUP)
        wide = jnp.dot(lat_v[r & 3, rows, :].astype(BF16), e_v[...], preferred_element_type=F32)
        wide = jnp.where(same_head(), wide, 0.0).astype(BF16)
        acc = acc + jnp.concatenate([jnp.dot(wide[i * GROUP:(i + 1) * GROUP], weights(w_ref, r, i),
                                             preferred_element_type=F32) for i in range(2)], axis=0)
        head_v[rows, :] = acc
        return jnp.where((r & 3) == 3, 0.0, acc)

    def setup(r, _):
        start_round(r, bwq, None)
        c = lax.broadcasted_iota(jnp.int32, (HD // NR, HD * HG), 0) + r * (HD // NR)
        col = lax.broadcasted_iota(jnp.int32, (HD // NR, HD * HG), 1)
        e_v[_tile(r, HD // NR), :] = jnp.where(c == col >> HG.bit_length() - 1, 1.0, 0.0).astype(BF16)

    _loop(NR, setup)
    x_copies = [pltpu.make_async_copy(ax_hbm, ax_v, x_sem.at[0]), pltpu.make_async_copy(bx_hbm, bx_v, x_sem.at[1])]
    for x_copy in x_copies:
        x_copy.start()
    _loop(NR, lambda r, _: start_round(r, wq, bwq))
    for x_copy in x_copies:
        x_copy.wait()
    xa = ax_v[...].astype(F32)
    for b in range(NB):
        for j in range(DM // HD):
            for g in range(NH // HG):
                lat_v[j, _tile(g * NB + b, HG), :] = jnp.broadcast_to(xa[b:b + 1, j * HD:(j + 1) * HD], (HG, HD))
    xb = bx_v[...].astype(F32)
    xb = jnp.concatenate([xb, xb], axis=0).astype(BF16)

    def b_queries(r, _):
        start_round(r, wuk, wq)
        cols = NH * HD // NR
        q = jnp.dot(xb, bwq_v[:, :, _tile(r, cols)].reshape(DM, cols), preferred_element_type=F32)
        for i in range(NH // NR):
            qb_v[r * (NH // NR) + i] = q[:, i * HD:(i + 1) * HD]

    wait_all(bwq_v, bwq_sem.at[0])
    _loop(NR, b_queries)

    def a_queries(r, acc):
        start_round(r, ckv(0), wuk)
        return up_project(wq_v, r, acc)

    wait_all(wq_v, wq_sem.at[0])
    _loop(NR, a_queries, jnp.zeros((2 * GROUP, HD), F32))

    def a_absorb(r, _):
        start_round(r, ckv(1), ckv(0))
        rows = _tile(r >> 2, 2 * GROUP)
        q = head_v[rows, :].astype(BF16)
        wide = jnp.concatenate([lax.dot_general(q[i * GROUP:(i + 1) * GROUP], weights(wuk_v, r, i), NT,
                                                preferred_element_type=F32) for i in range(2)], axis=0)
        wide = jnp.where(same_head(), wide, 0.0).astype(BF16)
        lat_v[r & 3, rows, :] = lax.dot_general(wide, e_v[...], NT, preferred_element_type=F32)

    wait_all(wuk_v, wuk_sem.at[0])
    _loop(NR, a_absorb)

    def a_attention(b, _):
        steps = NR // 2

        def start(r):
            pl.when(b < 2)(lambda: start_round(r, ckv(b + 2), ckv(b + 1)))
            pl.when(b == 2)(lambda: start_round(r, wuv, ckv(3)))
            pl.when(b == 3)(lambda: start_round(r, k_cache(0), wuv))

        def latents(i):
            return ckv_v[_tile(b * steps + i, SK // steps), :]

        heads = [_tile(g * NB + b, HG) for g in range(NH // HG)]
        q = jnp.concatenate([jnp.concatenate([lat_v[j, rows, :] for rows in heads], axis=0)
                             for j in range(DM // HD)], axis=1).astype(BF16)

        def scores(i, m):
            start(i)
            s = lax.dot_general(q, latents(i), NT, preferred_element_type=F32) * scale
            sa_v[i] = s
            return jnp.maximum(m, jnp.max(s, axis=-1, keepdims=True))

        def context(i, carry):
            start(steps + i)
            p = jnp.exp(sa_v[i] - m)
            c = jnp.dot(p.astype(BF16), latents(i), preferred_element_type=F32)
            return carry[0] + c, carry[1] + jnp.sum(p, axis=-1, keepdims=True)

        wait_all(ckv_v.at[_tile(b, SK)], ckv_sem.at[b])
        m = _loop(steps, scores, jnp.full((NH, 1), -jnp.inf, F32))
        c, l = _loop(steps, context, (jnp.zeros((NH, DM), F32), jnp.zeros((NH, 1), F32)))
        c = c / l
        for j in range(DM // HD):
            for g, rows in enumerate(heads):
                lat_v[j, rows, :] = c[g * HG:(g + 1) * HG, j * HD:(j + 1) * HD]

    _loop(NB, a_attention)

    def a_values(r, acc):
        start_round(r, v_cache(0), k_cache(0))
        return up_project(wuv_v, r, acc)

    wait_all(wuv_v, wuv_sem.at[0])
    _loop(NR, a_values, jnp.zeros((2 * GROUP, HD), F32))

    def b_head(h, _):
        step = SK // NR
        q = qb_v[h].astype(BF16)

        def batch(width):
            return lax.broadcasted_iota(jnp.int32, (2 * NB, width), 0) & (NB - 1)

        def wait_bulk(ref, sem):
            wait_all(ref.at[slot(h), :, pl.ds(0, SK - LATE)], sem.at[slot(h)])

        def wait_late(ref, sem, r):
            pl.when(r == NR - 1)(lambda: wait_all(ref.at[slot(h), :, pl.ds(SK - LATE, LATE)], sem.at[SLOTS + slot(h)]))

        def scores(r, m):
            pl.when(h + 1 < NH)(lambda: start_round(r, k_cache(h + 1), v_cache(h)))
            pl.when(h + 1 == NH)(lambda: start_round(r, wo, v_cache(NH - 1)))
            wait_late(k_v, k_sem, r)
            s = None
            for b in range(NB):
                d = lax.dot_general(q, k_v[slot(h), b, _tile(r, step), :], NT, preferred_element_type=F32)
                s = d if s is None else jnp.where(batch(step) == b, d, s)
            s = s * scale
            sb_v[r] = s
            return jnp.maximum(m, s)

        def context(r, carry):
            pl.when(h + 1 < NH)(lambda: start_round(r, v_cache(h + 1), k_cache(h + 1)))
            pl.when(h + 1 == NH)(lambda: start_round(r, bwo, wo))
            wait_late(v_v, v_sem, r)
            ctx, l = carry
            p = jnp.exp(sb_v[r] - m)
            for b in range(NB):
                d = jnp.dot(p.astype(BF16), v_v[slot(h), b, _tile(r, step), :], preferred_element_type=F32)
                ctx = ctx + jnp.where(batch(HD) == b, d, 0.0)
            return ctx, l + p

        wait_bulk(k_v, k_sem)
        m = jnp.max(_loop(NR, scores, jnp.full((2 * NB, step), -jnp.inf, F32)), axis=-1, keepdims=True)
        wait_bulk(v_v, v_sem)
        ctx, l = _loop(NR, context, (jnp.zeros((2 * NB, HD), F32), jnp.zeros((2 * NB, step), F32)))
        cb_v[h] = ctx / jnp.sum(l, axis=-1, keepdims=True)

    _loop(NH, b_head)
    for n in range(NS * NR - LAG, NS * NR):
        bwo(n % NS, n // NS, True)

    def a_output(i, acc):
        heads = NH // NR
        ctx = head_v[_tile(i >> 1, GROUP), :]
        head = lax.broadcasted_iota(jnp.int32, (GROUP, HD), 0) & (HG - 1)
        lhs = jnp.concatenate([jnp.where(head == (i & 1) * heads + j, ctx, 0.0) for j in range(heads)], axis=1)
        return acc + jnp.dot(lhs.astype(BF16), wo_v[_tile(i, heads * HD), :], preferred_element_type=F32)

    wait_all(wo_v, wo_sem.at[0])
    out_a = _loop(NR, a_output, jnp.zeros((GROUP, DM), F32))
    out_a = [jnp.sum(out_a[b * HG:(b + 1) * HG], axis=0, keepdims=True) for b in range(NB)]
    out_ref[:, pl.ds(0, DM)] = jnp.concatenate(out_a, axis=0).astype(out_ref.dtype)

    def b_output(i, streams, acc):
        for s in streams:
            acc = acc + jnp.dot(cb_v[s * (NH // NS) + i].astype(BF16), bwo_v[i, s], preferred_element_type=F32)
        return acc

    def b_outputs(i, acc):
        wait_all(bwo_v.at[i], bwo_sem.at[i])
        return b_output(i, range(NS), acc)

    out_b = _loop(3, b_outputs, jnp.zeros((2 * NB, DM), F32))
    for streams in (range(NS // 2), range(NS // 2, NS)):
        for s in streams:
            wait_all(bwo_v.at[3, s], bwo_sem.at[3 + s])
        out_b = b_output(3, streams, out_b)
    out_ref[:, pl.ds(DM, DM)] = out_b[:NB].astype(out_ref.dtype)


@jax.jit
def pallas_concat_heads__compressed_kv_cla__mha_block_cached__decode_kernel(
    A_x: jax.Array,
    A_c_kv: jax.Array,
    A_w_q: jax.Array,
    A_w_uk: jax.Array,
    A_w_uv: jax.Array,
    A_w_o: jax.Array,
    B_x: jax.Array,
    B_k_cache: jax.Array,
    B_v_cache: jax.Array,
    B_wq: jax.Array,
    B_wo: jax.Array,
):
    assert A_x.shape == (NB, 1, DM) and A_c_kv.shape == (NB, SK, DM) and A_w_q.shape == (DM, NH, HD)
    assert B_x.shape == (NB, 1, DM) and B_k_cache.shape == (NB, NH, SK, HD)
    scratch = [
        pltpu.VMEM((NB, DM), BF16),
        pltpu.VMEM((NB, DM), BF16),
        pltpu.VMEM((NB * SK, DM), BF16),
        pltpu.VMEM((DM, NH, HD), BF16),
        pltpu.VMEM((DM, NH, HD), BF16),
        pltpu.VMEM((DM, NH, HD), BF16),
        pltpu.VMEM((NH * HD, DM), BF16),
        pltpu.VMEM((DM // 8, 8, NH * HD), BF16),
        pltpu.VMEM((NH // NS, NS, HD, DM), BF16),
        pltpu.VMEM((SLOTS, NB, SK, HD), BF16),
        pltpu.VMEM((SLOTS, NB, SK, HD), BF16),
        pltpu.VMEM((HD, HD * HG), BF16),
        pltpu.VMEM((DM // HD, NB * NH, HD), F32),
        pltpu.VMEM((NB * NH, HD), F32),
        pltpu.VMEM((NR // 2, NH, 2 * SK // NR), F32),
        pltpu.VMEM((NH, 2 * NB, HD), F32),
        pltpu.VMEM((NR, 2 * NB, SK // NR), F32),
        pltpu.VMEM((NH, 2 * NB, HD), F32),
    ]
    out = pl.pallas_call(
        _kernel,
        out_shape=jax.ShapeDtypeStruct((NB, 2 * DM), A_x.dtype),
        in_specs=[pl.BlockSpec(memory_space=pl.ANY)] * 11,
        out_specs=pl.BlockSpec(memory_space=pltpu.VMEM),
        scratch_shapes=scratch,
        compiler_params=pltpu.CompilerParams(vmem_limit_bytes=100 * 1024 * 1024),
    )(
        A_x.reshape(NB, DM),
        A_c_kv.reshape(NB * SK, DM),
        A_w_q,
        A_w_uk,
        A_w_uv,
        A_w_o.reshape(NH * HD, DM),
        B_x.reshape(NB, DM),
        B_k_cache.reshape(NB * NH * SK, HD),
        B_v_cache.reshape(NB * NH * SK, HD),
        B_wq,
        B_wo,
    )
    return out.reshape(NB, 1, 2 * DM)
```
